```python
import jax
import jax.numpy as jnp

def _softmax(x, axis=-1):
    return jax.nn.softmax(x, axis=axis)
def _gelu(x):
    return jax.nn.gelu(x, approximate=True)
def _silu(x):
    return jax.nn.silu(x)
def _sigmoid(x):
    return jax.nn.sigmoid(x)
def _layernorm(x, axis=-1, eps=1e-5):
    m = jnp.mean(x, axis=axis, keepdims=True)
    v = jnp.var(x, axis=axis, keepdims=True)
    return (x - m) / jnp.sqrt(v + eps)
def _scatter_add(tgt, idx, src, axis=0):
    return tgt.at[idx].add(src)
def _segment_sum(src, seg, n):
    return jax.ops.segment_sum(src, seg, n)
class _Rng:
    def __init__(self, key):
        self._k = key
    def _next(self):
        self._k, sub = jax.random.split(self._k)
        return sub
    def normal(self, shape):
        return jax.random.normal(self._next(), shape, dtype=jnp.bfloat16)
    def randint(self, lo, hi, shape):
        return jax.random.randint(self._next(), shape, lo, hi, dtype=jnp.int32)
    def uniform(self, shape, lo=0.0, hi=1.0):
        return jax.random.uniform(self._next(), shape, jnp.bfloat16, lo, hi)
    def permutation(self, n):
        return jax.random.permutation(self._next(), n)


kernel_name = 'recurrent_scan__sliding_local_dilated__glu_gated_swiglu__prompt'

def setup_inputs():
    _rng = _Rng(jax.random.key(int.from_bytes(__import__("os").urandom(4), "little")))
    _w = (lambda a: (lambda t: t.astype(jnp.bfloat16) if jnp.issubdtype(t.dtype, jnp.floating) else t)(jnp.asarray(a)))
    def _A_setup():
        B, S, D = 1, 2048, 1024
        return {
            "x": _w((lambda *s: _rng.normal(s) * 0.05)(B, S, D)),
            "wqkv": _w((lambda *s: _rng.normal(s) * 0.05)(D, 3 * D)),
            "wo": _w((lambda *s: _rng.normal(s) * 0.05)(D, D)),
        }
    _A_in = _A_setup()

    def _B_setup():
        B, S, D, F = 1, 2048, 1024, 3584
        return {
            "x": _w((lambda *s: _rng.normal(s) * 0.05)(B, S, D)),
            "w1": _w((lambda *s: _rng.normal(s) * 0.05)(D, F) * (2.0 / D) ** 0.5),
            "w3": _w((lambda *s: _rng.normal(s) * 0.05)(D, F) * (2.0 / D) ** 0.5),
            "w2": _w((lambda *s: _rng.normal(s) * 0.05)(F, D) * (2.0 / F) ** 0.5),
        }
    _B_in = _B_setup()

    return {
        "A_x": _A_in["x"],
        "A_wqkv": _A_in["wqkv"],
        "A_wo": _A_in["wo"],
        "B_x": _B_in["x"],
        "B_w1": _B_in["w1"],
        "B_w3": _B_in["w3"],
        "B_w2": _B_in["w2"],
    }

def reference(A_x, A_wqkv, A_wo, B_x, B_w1, B_w3, B_w2):
    def _A_ref(x, wqkv, wo):
        B, S, D = x.shape
        H = 32; Dh = D // H
        W, dil = 8, 2
        qkv = (lambda x, *d: x.transpose(*d))((x @ wqkv).reshape(B, S, 3, H, Dh), 2, 0, 3, 1, 4)
        q, k, v = qkv[0], qkv[1], qkv[2]
        scale = Dh ** -0.5
        pos = jnp.arange(S)
        off = jnp.arange(W) * dil
        idx = pos[:, None] - off[None, :]
        mask = idx >= 0
        idx_c = jnp.where(mask, idx, 0).reshape(-1)
        kg = k[:, :, idx_c, :].reshape(B, H, S, W, Dh)
        vg = v[:, :, idx_c, :].reshape(B, H, S, W, Dh)
        logits = jnp.einsum("bhsd,bhswd->bhsw", q, kg) * scale
        logits = jnp.where(mask[None, None, :, :], logits, -1e9)
        attn = _softmax(logits, axis=-1)
        o = jnp.einsum("bhsw,bhswd->bhsd", attn, vg)
        return (lambda x, *d: x.transpose(*d))(o, 0, 2, 1, 3).reshape(B, S, D) @ wo

    def _B_ref(x, w1, w3, w2):
        gate = jnp.einsum("bsd,df->bsf", x, w1)
        up = jnp.einsum("bsd,df->bsf", x, w3)
        h = _silu(gate) * up
        out = jnp.einsum("bsf,fd->bsd", h, w2)
        return out

    x = A_x
    xn = _layernorm(x, axis=-1)
    s = _A_ref(xn, A_wqkv, A_wo)
    g = _silu(_B_ref(xn, B_w1, B_w3, B_w2))
    return x + s * g
```

```python
import functools

import jax
import jax.numpy as jnp
import jax.experimental.pallas as pl
import jax.experimental.pallas.tpu as pltpu

S = 2048
D = 1024
H = 32
DH = 32
W = 8
DIL = 2
F = 3584
LANES = 128
NT = D // LANES
HALO = 16

TM = 512
NSTEP = S // TM
FC = 896
NC = F // FC
RB = 16
AR = TM // NC

_F32 = jnp.float32
_BF16 = jnp.bfloat16
_NT_DIMS = (((1,), (1,)), ((), ()))


def _perm_matrix():
    m = jax.lax.broadcasted_iota(jnp.int32, (LANES, LANES), 0)
    c = jax.lax.broadcasted_iota(jnp.int32, (LANES, LANES), 1)
    i = m >> 4
    dd = (m >> 2) & 3
    hh = m & 3
    src = 32 * hh + 4 * i + dd
    return jnp.where(c == src, 1.0, 0.0).astype(_BF16)


def _group_allreduce(x, lane):
    hi8 = (lane & 8) != 0
    y = x + jnp.where(hi8, pltpu.roll(x, 8, 1), pltpu.roll(x, LANES - 8, 1))
    hi4 = (lane & 4) != 0
    return y + jnp.where(hi4, pltpu.roll(y, 4, 1), pltpu.roll(y, LANES - 4, 1))


def _layernorm(xb):
    x = xb.astype(_F32)
    mu = jnp.mean(x, axis=-1, keepdims=True)
    xc = x - mu
    var = jnp.mean(xc * xc, axis=-1, keepdims=True)
    return (xc * jax.lax.rsqrt(var + 1e-5)).astype(_BF16)


_SEM_X = 0
_SEM_QKV = _SEM_X + NSTEP
_SEM_WO = _SEM_QKV + 3
_SEM_F = _SEM_WO + 1
_NSEM = _SEM_F + 3 * NC


def _kernel(x_hbm, wqkv_hbm, wo_hbm, w1_hbm, w3_hbm, w2_hbm, out_ref,
            x_v, wqkv_v, wo_v, w1_v, w3_v, w2_v, wt_v, wop_v,
            xn_v, qkv_v, o_v, acc_v, sems):
    step = pl.program_id(0)
    cur = step % 2
    nxt = 1 - cur

    def x_copy(t):
        return pltpu.make_async_copy(
            x_hbm.at[pl.ds(t * TM, TM), :], x_v.at[t], sems.at[_SEM_X + t])

    def qkv_copy(p):
        return pltpu.make_async_copy(
            wqkv_hbm.at[:, pl.ds(p * D, D)], wqkv_v.at[p], sems.at[_SEM_QKV + p])

    def wo_copy():
        return pltpu.make_async_copy(wo_hbm, wo_v, sems.at[_SEM_WO])

    def f_copies(c):
        off = c * FC
        if not isinstance(c, int):
            off = pl.multiple_of(off, LANES)
        return [
            pltpu.make_async_copy(w1_hbm.at[:, pl.ds(off, FC)], w1_v.at[c], sems.at[_SEM_F + 3 * c]),
            pltpu.make_async_copy(w3_hbm.at[:, pl.ds(off, FC)], w3_v.at[c], sems.at[_SEM_F + 3 * c + 1]),
            pltpu.make_async_copy(w2_hbm.at[pl.ds(off, FC), :], w2_v.at[c], sems.at[_SEM_F + 3 * c + 2]),
        ]

    @pl.when(step == 0)
    def _():
        x_copy(0).start()
        for p in range(3):
            qkv_copy(p).start()
        for c in range(NC):
            for cp in f_copies(c):
                cp.start()
            if c == 0:
                for t in range(1, NSTEP):
                    x_copy(t).start()
            if c == NC - 2:
                wo_copy().start()
        for p in (1, 2):
            qkv_v[p, :, 0:HALO, :] = jnp.zeros((NT, HALO, LANES), _F32)
        x_copy(0).wait()
        xn_v[0] = _layernorm(x_v[0])

    @pl.when(step > 0)
    def _():
        for p in (1, 2):
            qkv_v[p, :, 0:HALO, :] = qkv_v[p, :, TM:TM + HALO, :]

    def qkv_body(p, carry):
        @pl.when(step == 0)
        def _():
            qkv_copy(pl.multiple_of(p, 1)).wait()
            P = _perm_matrix()
            for j in range(NT):
                m = wqkv_v[p, :, j * LANES:(j + 1) * LANES]
                t = jax.lax.dot_general(P, m, _NT_DIMS,
                                        preferred_element_type=_F32).astype(_BF16)
                for i in range(NT):
                    wt_v[p, i * LANES + 16 * j:i * LANES + 16 * j + 16, :] = t[16 * i:16 * i + 16, :]

        r = jax.lax.dot_general(xn_v[cur], wt_v[p], _NT_DIMS, preferred_element_type=_F32)
        for i in range(NT):
            qkv_v[p, i, HALO:HALO + TM, :] = r[:, i * LANES:(i + 1) * LANES]
        return carry

    jax.lax.fori_loop(0, 3, qkv_body, 0)

    lane = jax.lax.broadcasted_iota(jnp.int32, (RB, LANES), 1)
    row = jax.lax.broadcasted_iota(jnp.int32, (RB, LANES), 0)
    scale = DH ** -0.5

    def attn_block(r0):
        grow = row + (step * TM + r0)
        qs = [qkv_v[0, i, pl.ds(r0 + HALO, RB), :] for i in range(NT)]
        logits = []
        for w in range(W):
            acc = None
            for i in range(NT):
                p = qs[i] * qkv_v[1, i, pl.ds(r0 + HALO - DIL * w, RB), :]
                acc = p if acc is None else acc + p
            l = _group_allreduce(acc, lane) * scale
            if w > 0:
                l = jnp.where(grow >= DIL * w, l, -1e9)
            logits.append(l)
        mx = logits[0]
        for w in range(1, W):
            mx = jnp.maximum(mx, logits[w])
        es = [jnp.exp(l - mx) for l in logits]
        den = es[0]
        for w in range(1, W):
            den = den + es[w]
        inv = 1.0 / den
        ps = [e * inv for e in es]
        for i in range(NT):
            acc = None
            for w in range(W):
                p = ps[w] * qkv_v[2, i, pl.ds(r0 + HALO - DIL * w, RB), :]
                acc = p if acc is None else acc + p
            o_v[pl.ds(r0, RB), i * LANES:(i + 1) * LANES] = acc.astype(_BF16)

    def ffn_body(c, carry):
        @pl.when(step == 0)
        def _():
            for cp in f_copies(c):
                cp.wait()

        @pl.when(jnp.logical_and(c == 0, step < NSTEP - 1))
        def _():
            x_copy(step + 1).wait()

        xn = xn_v[cur]
        gate = jnp.dot(xn, w1_v[c], preferred_element_type=_F32)
        up = jnp.dot(xn, w3_v[c], preferred_element_type=_F32)
        h = (gate * jax.nn.sigmoid(gate) * up).astype(_BF16)
        d = jnp.dot(h, w2_v[c], preferred_element_type=_F32)
        acc_v[...] = jnp.where(c > 0, acc_v[...], 0.0) + d

        base = pl.multiple_of(c * AR, AR)
        for b in range(AR // RB):
            attn_block(base + b * RB)
        nt = jnp.minimum(step + 1, NSTEP - 1)
        xn_v[nxt, pl.ds(base, AR), :] = _layernorm(x_v[nt, pl.ds(base, AR), :])
        return carry

    jax.lax.fori_loop(0, NC, ffn_body, 0)

    @pl.when(step == 0)
    def _():
        wo_copy().wait()
        P = _perm_matrix()
        for j in range(NT):
            t = jnp.dot(P, wo_v[j * LANES:(j + 1) * LANES, :],
                        preferred_element_type=_F32).astype(_BF16)
            for i in range(NT):
                wop_v[i * LANES + 16 * j:i * LANES + 16 * j + 16, :] = t[16 * i:16 * i + 16, :]

    ffn = acc_v[...]
    g = ffn * jax.nn.sigmoid(ffn)
    s = jnp.dot(o_v[...], wop_v[...], preferred_element_type=_F32)
    out_ref[...] = (x_v[step].astype(_F32) + s * g).astype(out_ref.dtype)


@jax.jit
def pallas_recurrent_scan__sliding_local_dilated__glu_gated_swiglu__prompt_kernel(
    A_x: jax.Array,
    A_wqkv: jax.Array,
    A_wo: jax.Array,
    B_x: jax.Array,
    B_w1: jax.Array,
    B_w3: jax.Array,
    B_w2: jax.Array,
):
    x = A_x.reshape(S, D)
    any_spec = pl.BlockSpec(memory_space=pl.ANY)
    out = pl.pallas_call(
        _kernel,
        grid=(NSTEP,),
        in_specs=[any_spec] * 6,
        out_specs=pl.BlockSpec((TM, D), lambda i: (i, 0)),
        out_shape=jax.ShapeDtypeStruct((S, D), A_x.dtype),
        scratch_shapes=[
            pltpu.VMEM((NSTEP, TM, D), _BF16),
            pltpu.VMEM((3, D, D), _BF16),
            pltpu.VMEM((D, D), _BF16),
            pltpu.VMEM((NC, D, FC), _BF16),
            pltpu.VMEM((NC, D, FC), _BF16),
            pltpu.VMEM((NC, FC, D), _BF16),
            pltpu.VMEM((3, D, D), _BF16),
            pltpu.VMEM((D, D), _BF16),
            pltpu.VMEM((2, TM, D), _BF16),
            pltpu.VMEM((3, NT, TM + HALO, LANES), _F32),
            pltpu.VMEM((TM, D), _BF16),
            pltpu.VMEM((TM, D), _F32),
            pltpu.SemaphoreType.DMA((_NSEM,)),
        ],
        compiler_params=pltpu.CompilerParams(
            dimension_semantics=("arbitrary",),
            vmem_limit_bytes=110 * 1024 * 1024,
        ),
        name="fused_block",
    )(x, A_wqkv, A_wo, B_w1, B_w3, B_w2)
    return out.reshape(A_x.shape)
```

```python
import functools

import jax
import jax.numpy as jnp
import jax.experimental.pallas as pl
import jax.experimental.pallas.tpu as pltpu

S = 2048
D = 1024
H = 32
DH = 32
W = 8
DIL = 2
F = 3584
LANES = 128
NT = D // LANES
HALO = 16

TM = 512
NSTEP = S // TM
FC = 896
NC = F // FC
RB = 8
AR = TM // NC
QCH = 8
XCH = 4
PR = 128

_F32 = jnp.float32
_BF16 = jnp.bfloat16
_U32 = jnp.uint32


def _xor_lanes(x, k):
    lane = jax.lax.broadcasted_iota(jnp.int32, x.shape, 1)
    return jnp.take_along_axis(x, lane ^ k, axis=1)


def _lane_butterfly(tiles, use_perm=False):
    s = list(tiles)
    lane = jax.lax.broadcasted_iota(jnp.int32, s[0].shape, 1)
    for b in range(3):
        sh = 4 << b
        lo = (lane & sh) == 0
        ns = list(s)
        for a in range(NT):
            if a & (1 << b):
                continue
            c = a | (1 << b)
            if use_perm:
                r = _xor_lanes(jnp.where(lo, s[c], s[a]), sh)
                ns[a] = jnp.where(lo, s[a], r)
                ns[c] = jnp.where(lo, r, s[c])
            else:
                ns[a] = jnp.where(lo, s[a], pltpu.roll(s[c], sh, 1))
                ns[c] = jnp.where(lo, pltpu.roll(s[a], LANES - sh, 1), s[c])
        s = ns
    return s


def _prep_cols(src, dst, r0, nrows, use_perm=False):
    for r in range(r0, r0 + nrows, PR):
        outs = _lane_butterfly([pltpu.bitcast(src[r:r + PR, j * LANES:(j + 1) * LANES], _U32)
                                for j in range(NT)], use_perm)
        for i in range(NT):
            dst[i, r // 2:(r + PR) // 2, :] = outs[i]


def _layernorm(xb):
    x = xb.astype(_F32)
    mu = jnp.mean(x, axis=-1, keepdims=True)
    xc = x - mu
    var = jnp.mean(xc * xc, axis=-1, keepdims=True)
    return (xc * jax.lax.rsqrt(var + 1e-5)).astype(_BF16)


_SEM_X = 0
_SEM_X0 = _SEM_X + NSTEP
_SEM_Q = _SEM_X0 + XCH
_SEM_K = _SEM_Q + QCH
_SEM_V = _SEM_K + 1
_SEM_WO = _SEM_V + 1
_SEM_F = _SEM_WO + 1
_NSEM = _SEM_F + 3 * NC


def _kernel(x_hbm, wqkv_hbm, wo_hbm, w1_hbm, w3_hbm, w2_hbm, out_ref,
            x_v, wqkv_v, wo_v, w1_v, w3_v, w2_v, wq_p, wk_p, wv_p,
            xn_v, q_v, k_v, v_v, o_v, acc_v, sems):
    step = pl.program_id(0)
    cur = step % 2
    nxt = 1 - cur
    QR = D // QCH

    def x_copy(t):
        return pltpu.make_async_copy(
            x_hbm.at[pl.ds(t * TM, TM), :], x_v.at[t], sems.at[_SEM_X + t])

    def x0_copy(ch):
        n = TM // XCH
        return pltpu.make_async_copy(
            x_hbm.at[pl.ds(ch * n, n), :], x_v.at[0, pl.ds(ch * n, n), :], sems.at[_SEM_X0 + ch])

    def q_copy(ch):
        return pltpu.make_async_copy(
            wqkv_hbm.at[pl.ds(ch * QR, QR), pl.ds(0, D)],
            wqkv_v.at[0, pl.ds(ch * QR, QR), :], sems.at[_SEM_Q + ch])

    def kv_copy(p):
        return pltpu.make_async_copy(
            wqkv_hbm.at[:, pl.ds(p * D, D)], wqkv_v.at[p], sems.at[_SEM_K + p - 1])

    def wo_copy():
        return pltpu.make_async_copy(wo_hbm, wo_v, sems.at[_SEM_WO])

    def f_copies(c):
        off = c * FC
        if not isinstance(c, int):
            off = pl.multiple_of(off, LANES)
        return [
            pltpu.make_async_copy(w1_hbm.at[:, pl.ds(off, FC)], w1_v.at[c], sems.at[_SEM_F + 3 * c]),
            pltpu.make_async_copy(w3_hbm.at[:, pl.ds(off, FC)], w3_v.at[c], sems.at[_SEM_F + 3 * c + 1]),
            pltpu.make_async_copy(w2_hbm.at[pl.ds(off, FC), :], w2_v.at[c], sems.at[_SEM_F + 3 * c + 2]),
        ]

    @pl.when(step == 0)
    def _():
        order = "qqqxqqxqqxqx"
        nq = nx = 0
        for kind in order:
            if kind == "q":
                q_copy(nq).start()
                nq += 1
            else:
                x0_copy(nx).start()
                nx += 1
        kv_copy(1).start()
        kv_copy(2).start()
        for c in range(NC):
            for cp in f_copies(c):
                cp.start()
            if c == 0:
                x_copy(1).start()
            if c == 1:
                wo_copy().start()
                for t in range(2, NSTEP):
                    x_copy(t).start()
        nq = nx = 0
        for kind in order:
            if kind == "q":
                q_copy(nq).wait()
                _prep_cols(wqkv_v.at[0], wq_p, nq * QR, QR, True)
                nq += 1
            else:
                n = TM // XCH
                x0_copy(nx).wait()
                xn_v[0, nx * n:(nx + 1) * n, :] = _layernorm(x_v[0, nx * n:(nx + 1) * n, :])
                nx += 1

    first = step == 0
    for buf in (k_v, v_v):
        buf[:, 0:HALO, :] = jnp.where(first, 0.0, buf[:, TM:TM + HALO, :])
    xn = xn_v[cur]
    for i in range(NT // 2):
        q_v[i] = jnp.dot(xn, pltpu.bitcast(wq_p[i], _BF16), preferred_element_type=_F32)

    @pl.when(step == 0)
    def _():
        kv_copy(1).wait()

    xn = xn_v[cur]
    for i in range(NT // 2, NT):
        q_v[i] = jnp.dot(xn, pltpu.bitcast(wq_p[i], _BF16), preferred_element_type=_F32)
    _prep_cols(wqkv_v.at[1], wk_p, 0, D, True)

    @pl.when(step == 0)
    def _():
        kv_copy(2).wait()

    xn = xn_v[cur]
    for i in range(NT):
        k_v[i, HALO:HALO + TM, :] = jnp.dot(xn, pltpu.bitcast(wk_p[i], _BF16), preferred_element_type=_F32)
    _prep_cols(wqkv_v.at[2], wv_p, 0, D)

    xn = xn_v[cur]
    for i in range(NT):
        v_v[i, HALO:HALO + TM, :] = jnp.dot(xn, pltpu.bitcast(wv_p[i], _BF16), preferred_element_type=_F32)

    row = jax.lax.broadcasted_iota(jnp.int32, (RB, LANES), 0)
    scale = DH ** -0.5
    lane = jax.lax.broadcasted_iota(jnp.int32, (RB, LANES), 1)
    odd1 = (lane & 1) != 0
    odd2 = (lane & 2) != 0

    def attn_block(r0):
        grow = row + (step * TM + r0)
        qs = [q_v[i, pl.ds(r0, RB), :] for i in range(NT)]
        logits = []
        for w in range(W):
            acc = None
            for i in range(NT):
                p = qs[i] * k_v[i, pl.ds(r0 + HALO - DIL * w, RB), :]
                acc = p if acc is None else acc + p
            acc = acc + jnp.where(odd1, pltpu.roll(acc, 1, 1), pltpu.roll(acc, LANES - 1, 1))
            acc = acc + jnp.where(odd2, pltpu.roll(acc, 2, 1), pltpu.roll(acc, LANES - 2, 1))
            l = acc * scale
            if w > 0:
                l = jnp.where(grow >= DIL * w, l, -1e9)
            logits.append(l)
        mx = logits[0]
        for w in range(1, W):
            mx = jnp.maximum(mx, logits[w])
        es = [jnp.exp(l - mx) for l in logits]
        den = es[0]
        for w in range(1, W):
            den = den + es[w]
        inv = 1.0 / den
        ps = [e * inv for e in es]
        os_ = []
        for i in range(NT):
            acc = None
            for w in range(W):
                p = ps[w] * v_v[i, pl.ds(r0 + HALO - DIL * w, RB), :]
                acc = p if acc is None else acc + p
            os_.append(acc)
        os_ = _lane_butterfly(os_)
        for i in range(NT):
            o_v[pl.ds(r0, RB), i * LANES:(i + 1) * LANES] = os_[i].astype(_BF16)

    def ffn_body(c, carry):
        @pl.when(step == 0)
        def _():
            for cp in f_copies(c):
                cp.wait()

        @pl.when(jnp.logical_and(c == 0, step < NSTEP - 1))
        def _():
            x_copy(step + 1).wait()

        xn = xn_v[cur]
        gate = jnp.dot(xn, w1_v[c], preferred_element_type=_F32)
        up = jnp.dot(xn, w3_v[c], preferred_element_type=_F32)
        h = (gate * jax.nn.sigmoid(gate) * up).astype(_BF16)
        d = jnp.dot(h, w2_v[c], preferred_element_type=_F32)
        acc_v[...] = jnp.where(c > 0, acc_v[...], 0.0) + d

        base = pl.multiple_of(c * AR, AR)
        for b in range(AR // RB):
            attn_block(base + b * RB)
        nt = jnp.minimum(step + 1, NSTEP - 1)
        xn_v[nxt, pl.ds(base, AR), :] = _layernorm(x_v[nt, pl.ds(base, AR), :])
        return carry

    jax.lax.fori_loop(0, NC, ffn_body, 0)

    @pl.when(step == 0)
    def _():
        wo_copy().wait()

    o = o_v[...]
    for ct in range(NT):
        cols = slice(ct * LANES, (ct + 1) * LANES)
        s = jnp.dot(o, wo_v[:, cols], preferred_element_type=_F32)
        ffn = acc_v[:, cols]
        g = ffn * jax.nn.sigmoid(ffn)
        out_ref[:, cols] = (x_v[step, :, cols].astype(_F32) + s * g).astype(out_ref.dtype)


@jax.jit
def pallas_recurrent_scan__sliding_local_dilated__glu_gated_swiglu__prompt_kernel(
    A_x: jax.Array,
    A_wqkv: jax.Array,
    A_wo: jax.Array,
    B_x: jax.Array,
    B_w1: jax.Array,
    B_w3: jax.Array,
    B_w2: jax.Array,
):
    x = A_x.reshape(S, D)
    any_spec = pl.BlockSpec(memory_space=pl.ANY)
    wp = pltpu.VMEM((NT, D // 2, LANES), _U32)
    out = pl.pallas_call(
        _kernel,
        grid=(NSTEP,),
        in_specs=[any_spec] * 6,
        out_specs=pl.BlockSpec((TM, D), lambda i: (i, 0)),
        out_shape=jax.ShapeDtypeStruct((S, D), A_x.dtype),
        scratch_shapes=[
            pltpu.VMEM((NSTEP, TM, D), _BF16),
            pltpu.VMEM((3, D, D), _BF16),
            pltpu.VMEM((D, D), _BF16),
            pltpu.VMEM((NC, D, FC), _BF16),
            pltpu.VMEM((NC, D, FC), _BF16),
            pltpu.VMEM((NC, FC, D), _BF16),
            wp, wp, wp,
            pltpu.VMEM((2, TM, D), _BF16),
            pltpu.VMEM((NT, TM, LANES), _F32),
            pltpu.VMEM((NT, TM + HALO, LANES), _F32),
            pltpu.VMEM((NT, TM + HALO, LANES), _F32),
            pltpu.VMEM((TM, D), _BF16),
            pltpu.VMEM((TM, D), _F32),
            pltpu.SemaphoreType.DMA((_NSEM,)),
        ],
        compiler_params=pltpu.CompilerParams(
            dimension_semantics=("arbitrary",),
            vmem_limit_bytes=110 * 1024 * 1024,
        ),
        name="fused_block",
    )(x, A_wqkv, A_wo, B_w1, B_w3, B_w2)
    return out.reshape(A_x.shape)
```

```python
import functools

import jax
import jax.numpy as jnp
import jax.experimental.pallas as pl
import jax.experimental.pallas.tpu as pltpu

S = 2048
D = 1024
H = 32
DH = 32
W = 8
DIL = 2
F = 3584
LANES = 128
NT = D // LANES
HALO = 16

TM = 512
NSTEP = S // TM
FC = 896
NC = F // FC
RB = 8
AR = TM // NC
QCH = 8
OCH = 8
XCH = 4
PR = 128

_F32 = jnp.float32
_BF16 = jnp.bfloat16
_U32 = jnp.uint32


def _xor_lanes(x, k):
    lane = jax.lax.broadcasted_iota(jnp.int32, x.shape, 1)
    return jnp.take_along_axis(x, lane ^ k, axis=1)


def _lane_butterfly(tiles, use_perm=False):
    s = list(tiles)
    lane = jax.lax.broadcasted_iota(jnp.int32, s[0].shape, 1)
    for b in range(3):
        sh = 4 << b
        lo = (lane & sh) == 0
        ns = list(s)
        for a in range(NT):
            if a & (1 << b):
                continue
            c = a | (1 << b)
            if use_perm:
                r = _xor_lanes(jnp.where(lo, s[c], s[a]), sh)
                ns[a] = jnp.where(lo, s[a], r)
                ns[c] = jnp.where(lo, r, s[c])
            else:
                ns[a] = jnp.where(lo, s[a], pltpu.roll(s[c], sh, 1))
                ns[c] = jnp.where(lo, pltpu.roll(s[a], LANES - sh, 1), s[c])
        s = ns
    return s


def _prep_cols(src, dst, r0, nrows, use_perm=False):
    for r in range(r0, r0 + nrows, PR):
        outs = _lane_butterfly([pltpu.bitcast(src[r:r + PR, j * LANES:(j + 1) * LANES], _U32)
                                for j in range(NT)], use_perm)
        for i in range(NT):
            dst[i, r // 2:(r + PR) // 2, :] = outs[i]


def _layernorm(xb):
    x = xb.astype(_F32)
    mu = jnp.mean(x, axis=-1, keepdims=True)
    xc = x - mu
    var = jnp.mean(xc * xc, axis=-1, keepdims=True)
    return (xc * jax.lax.rsqrt(var + 1e-5)).astype(_BF16)


_SEM_X = 0
_SEM_X0 = _SEM_X + NSTEP
_SEM_Q = _SEM_X0 + XCH
_SEM_K = _SEM_Q + QCH
_SEM_V = _SEM_K + 1
_SEM_WO = _SEM_V + 1
_SEM_F = _SEM_WO + 1
_SEM_OUT = _SEM_F + 3 * NC
_NSEM = _SEM_OUT + OCH


def _kernel(x_hbm, wqkv_hbm, wo_hbm, w1_hbm, w3_hbm, w2_hbm, out_hbm,
            x_v, wqkv_v, wo_v, w1_v, w3_v, w2_v, wq_p, wk_p, wv_p,
            xn_v, q_v, k_v, v_v, o_v, acc_v, out_v, sems):
    step = pl.program_id(0)
    cur = step % 2
    nxt = 1 - cur
    QR = D // QCH

    def x_copy(t):
        return pltpu.make_async_copy(
            x_hbm.at[pl.ds(t * TM, TM), :], x_v.at[t], sems.at[_SEM_X + t])

    def x0_copy(ch):
        n = TM // XCH
        return pltpu.make_async_copy(
            x_hbm.at[pl.ds(ch * n, n), :], x_v.at[0, pl.ds(ch * n, n), :], sems.at[_SEM_X0 + ch])

    def q_copy(ch):
        return pltpu.make_async_copy(
            wqkv_hbm.at[pl.ds(ch * QR, QR), pl.ds(0, D)],
            wqkv_v.at[0, pl.ds(ch * QR, QR), :], sems.at[_SEM_Q + ch])

    def kv_copy(p):
        return pltpu.make_async_copy(
            wqkv_hbm.at[:, pl.ds(p * D, D)], wqkv_v.at[p], sems.at[_SEM_K + p - 1])

    def wo_copy():
        return pltpu.make_async_copy(wo_hbm, wo_v, sems.at[_SEM_WO])

    def f_copies(c):
        off = c * FC
        if not isinstance(c, int):
            off = pl.multiple_of(off, LANES)
        return [
            pltpu.make_async_copy(w1_hbm.at[:, pl.ds(off, FC)], w1_v.at[c], sems.at[_SEM_F + 3 * c]),
            pltpu.make_async_copy(w3_hbm.at[:, pl.ds(off, FC)], w3_v.at[c], sems.at[_SEM_F + 3 * c + 1]),
            pltpu.make_async_copy(w2_hbm.at[pl.ds(off, FC), :], w2_v.at[c], sems.at[_SEM_F + 3 * c + 2]),
        ]

    @pl.when(step == 0)
    def _():
        order = "qqqxqqxqqxqx"
        nq = nx = 0
        for kind in order:
            if kind == "q":
                q_copy(nq).start()
                nq += 1
            else:
                x0_copy(nx).start()
                nx += 1
        kv_copy(1).start()
        kv_copy(2).start()
        for c in range(NC):
            for cp in f_copies(c):
                cp.start()
            if c == 0:
                x_copy(1).start()
            if c == 1:
                wo_copy().start()
                for t in range(2, NSTEP):
                    x_copy(t).start()
        nq = nx = 0
        for kind in order:
            if kind == "q":
                q_copy(nq).wait()
                _prep_cols(wqkv_v.at[0], wq_p, nq * QR, QR, True)
                nq += 1
            else:
                n = TM // XCH
                x0_copy(nx).wait()
                xn_v[0, nx * n:(nx + 1) * n, :] = _layernorm(x_v[0, nx * n:(nx + 1) * n, :])
                nx += 1

    first = step == 0
    for buf in (k_v, v_v):
        buf[:, 0:HALO, :] = jnp.where(first, 0.0, buf[:, TM:TM + HALO, :])
    xn = xn_v[cur]
    for i in range(NT // 2):
        q_v[i] = jnp.dot(xn, pltpu.bitcast(wq_p[i], _BF16), preferred_element_type=_F32)

    @pl.when(step == 0)
    def _():
        kv_copy(1).wait()

    xn = xn_v[cur]
    for i in range(NT // 2, NT):
        q_v[i] = jnp.dot(xn, pltpu.bitcast(wq_p[i], _BF16), preferred_element_type=_F32)
    _prep_cols(wqkv_v.at[1], wk_p, 0, D, True)

    @pl.when(step == 0)
    def _():
        kv_copy(2).wait()

    xn = xn_v[cur]
    for i in range(NT):
        k_v[i, HALO:HALO + TM, :] = jnp.dot(xn, pltpu.bitcast(wk_p[i], _BF16), preferred_element_type=_F32)
    _prep_cols(wqkv_v.at[2], wv_p, 0, D)

    xn = xn_v[cur]
    for i in range(NT):
        v_v[i, HALO:HALO + TM, :] = jnp.dot(xn, pltpu.bitcast(wv_p[i], _BF16), preferred_element_type=_F32)

    row = jax.lax.broadcasted_iota(jnp.int32, (RB, LANES), 0)
    scale = DH ** -0.5
    lane = jax.lax.broadcasted_iota(jnp.int32, (RB, LANES), 1)
    odd1 = (lane & 1) != 0
    odd2 = (lane & 2) != 0

    def attn_block(r0):
        grow = row + (step * TM + r0)
        qs = [q_v[i, pl.ds(r0, RB), :] for i in range(NT)]
        logits = []
        for w in range(W):
            acc = None
            for i in range(NT):
                p = qs[i] * k_v[i, pl.ds(r0 + HALO - DIL * w, RB), :]
                acc = p if acc is None else acc + p
            acc = acc + jnp.where(odd1, pltpu.roll(acc, 1, 1), pltpu.roll(acc, LANES - 1, 1))
            acc = acc + jnp.where(odd2, pltpu.roll(acc, 2, 1), pltpu.roll(acc, LANES - 2, 1))
            l = acc * scale
            if w > 0:
                l = jnp.where(grow >= DIL * w, l, -1e9)
            logits.append(l)
        mx = logits[0]
        for w in range(1, W):
            mx = jnp.maximum(mx, logits[w])
        es = [jnp.exp(l - mx) for l in logits]
        den = es[0]
        for w in range(1, W):
            den = den + es[w]
        inv = 1.0 / den
        ps = [e * inv for e in es]
        os_ = []
        for i in range(NT):
            acc = None
            for w in range(W):
                p = ps[w] * v_v[i, pl.ds(r0 + HALO - DIL * w, RB), :]
                acc = p if acc is None else acc + p
            os_.append(acc)
        os_ = _lane_butterfly(os_)
        for i in range(NT):
            o_v[pl.ds(r0, RB), i * LANES:(i + 1) * LANES] = os_[i].astype(_BF16)

    def ffn_body(c, carry):
        @pl.when(step == 0)
        def _():
            for cp in f_copies(c):
                cp.wait()

        @pl.when(jnp.logical_and(c == 0, step < NSTEP - 1))
        def _():
            x_copy(step + 1).wait()

        xn = xn_v[cur]
        gate = jnp.dot(xn, w1_v[c], preferred_element_type=_F32)
        up = jnp.dot(xn, w3_v[c], preferred_element_type=_F32)
        h = (gate * jax.nn.sigmoid(gate) * up).astype(_BF16)
        d = jnp.dot(h, w2_v[c], preferred_element_type=_F32)
        acc_v[...] = jnp.where(c > 0, acc_v[...], 0.0) + d

        base = pl.multiple_of(c * AR, AR)
        for b in range(AR // RB):
            attn_block(base + b * RB)
        nt = jnp.minimum(step + 1, NSTEP - 1)
        xn_v[nxt, pl.ds(base, AR), :] = _layernorm(x_v[nt, pl.ds(base, AR), :])
        return carry

    jax.lax.fori_loop(0, NC, ffn_body, 0)

    @pl.when(step == 0)
    def _():
        wo_copy().wait()

    OC = D // OCH

    def out_copy(t, ch):
        return pltpu.make_async_copy(
            out_v.at[ch], out_hbm.at[pl.ds(t * TM, TM), pl.ds(ch * OC, OC)],
            sems.at[_SEM_OUT + ch])

    @pl.when(step > 0)
    def _():
        for ch in range(OCH):
            out_copy(step - 1, ch).wait()

    o = o_v[...]
    for ct in range(NT):
        cols = slice(ct * LANES, (ct + 1) * LANES)
        s = jnp.dot(o, wo_v[:, cols], preferred_element_type=_F32)
        ffn = acc_v[:, cols]
        g = ffn * jax.nn.sigmoid(ffn)
        per = NT // OCH
        ch, sub = ct // per, ct % per
        out_v[ch, :, sub * LANES:(sub + 1) * LANES] = (
            x_v[step, :, cols].astype(_F32) + s * g).astype(out_v.dtype)
        if sub == per - 1:
            out_copy(step, ch).start()

    @pl.when(step == NSTEP - 1)
    def _():
        for ch in range(OCH):
            out_copy(step, ch).wait()


@jax.jit
def pallas_recurrent_scan__sliding_local_dilated__glu_gated_swiglu__prompt_kernel(
    A_x: jax.Array,
    A_wqkv: jax.Array,
    A_wo: jax.Array,
    B_x: jax.Array,
    B_w1: jax.Array,
    B_w3: jax.Array,
    B_w2: jax.Array,
):
    x = A_x.reshape(S, D)
    any_spec = pl.BlockSpec(memory_space=pl.ANY)
    wp = pltpu.VMEM((NT, D // 2, LANES), _U32)
    out = pl.pallas_call(
        _kernel,
        grid=(NSTEP,),
        in_specs=[any_spec] * 6,
        out_specs=any_spec,
        out_shape=jax.ShapeDtypeStruct((S, D), A_x.dtype),
        scratch_shapes=[
            pltpu.VMEM((NSTEP, TM, D), _BF16),
            pltpu.VMEM((3, D, D), _BF16),
            pltpu.VMEM((D, D), _BF16),
            pltpu.VMEM((NC, D, FC), _BF16),
            pltpu.VMEM((NC, D, FC), _BF16),
            pltpu.VMEM((NC, FC, D), _BF16),
            wp, wp, wp,
            pltpu.VMEM((2, TM, D), _BF16),
            pltpu.VMEM((NT, TM, LANES), _F32),
            pltpu.VMEM((NT, TM + HALO, LANES), _F32),
            pltpu.VMEM((NT, TM + HALO, LANES), _F32),
            pltpu.VMEM((TM, D), _BF16),
            pltpu.VMEM((TM, D), _F32),
            pltpu.VMEM((OCH, TM, D // OCH), _BF16),
            pltpu.SemaphoreType.DMA((_NSEM,)),
        ],
        compiler_params=pltpu.CompilerParams(
            dimension_semantics=("arbitrary",),
            vmem_limit_bytes=110 * 1024 * 1024,
        ),
        name="fused_block",
    )(x, A_wqkv, A_wo, B_w1, B_w3, B_w2)
    return out.reshape(A_x.shape)
```

```python
import functools

import jax
import jax.numpy as jnp
import jax.experimental.pallas as pl
import jax.experimental.pallas.tpu as pltpu

S = 2048
D = 1024
H = 32
DH = 32
W = 8
DIL = 2
F = 3584
LANES = 128
NT = D // LANES
HALO = 16

TM = 512
NSTEP = S // TM
FC = 896
NC = F // FC
RB = 8
AR = TM // NC
QCH = 8
OCH = 8
XCH = 4
PR = 128

_F32 = jnp.float32
_BF16 = jnp.bfloat16
_U32 = jnp.uint32


def _xor_lanes(x, k):
    lane = jax.lax.broadcasted_iota(jnp.int32, x.shape, 1)
    return jnp.take_along_axis(x, lane ^ k, axis=1)


def _lane_butterfly(tiles, use_perm=False):
    s = list(tiles)
    lane = jax.lax.broadcasted_iota(jnp.int32, s[0].shape, 1)
    for b in range(3):
        sh = 4 << b
        lo = (lane & sh) == 0
        ns = list(s)
        for a in range(NT):
            if a & (1 << b):
                continue
            c = a | (1 << b)
            if use_perm:
                r = _xor_lanes(jnp.where(lo, s[c], s[a]), sh)
                ns[a] = jnp.where(lo, s[a], r)
                ns[c] = jnp.where(lo, r, s[c])
            else:
                ns[a] = jnp.where(lo, s[a], pltpu.roll(s[c], sh, 1))
                ns[c] = jnp.where(lo, pltpu.roll(s[a], LANES - sh, 1), s[c])
        s = ns
    return s


def _prep_cols(src, dst, r0, nrows, use_perm=False):
    for r in range(r0, r0 + nrows, PR):
        outs = _lane_butterfly([pltpu.bitcast(src[r:r + PR, j * LANES:(j + 1) * LANES], _U32)
                                for j in range(NT)], use_perm)
        for i in range(NT):
            dst[i, r // 2:(r + PR) // 2, :] = outs[i]


def _layernorm(xb):
    x = xb.astype(_F32)
    mu = jnp.mean(x, axis=-1, keepdims=True)
    xc = x - mu
    var = jnp.mean(xc * xc, axis=-1, keepdims=True)
    return (xc * jax.lax.rsqrt(var + 1e-5)).astype(_BF16)


_SEM_X = 0
_SEM_X0 = _SEM_X + NSTEP
_SEM_QK = _SEM_X0 + XCH
_SEM_V = _SEM_QK + 4
_SEM_WO = _SEM_V + 1
_SEM_F = _SEM_WO + 1
_SEM_OUT = _SEM_F + 3 * NC
_NSEM = _SEM_OUT + OCH


def _kernel(x_hbm, wqkv_hbm, wo_hbm, w1_hbm, w3_hbm, w2_hbm, out_hbm,
            x_v, wqk_v, wv_v, wo_v, w1_v, w3_v, w2_v, wv_p,
            xn_v, q_v, k_v, v_v, o_v, acc_v, out_v, sems):
    step = pl.program_id(0)
    cur = step % 2
    nxt = 1 - cur
    QR = D // QCH

    def x_copy(t):
        return pltpu.make_async_copy(
            x_hbm.at[pl.ds(t * TM, TM), :], x_v.at[t], sems.at[_SEM_X + t])

    def x0_copy(ch):
        n = TM // XCH
        return pltpu.make_async_copy(
            x_hbm.at[pl.ds(ch * n, n), :], x_v.at[0, pl.ds(ch * n, n), :], sems.at[_SEM_X0 + ch])

    def qk_copy(n):
        p, hf = n // 2, n % 2
        return pltpu.make_async_copy(
            wqkv_hbm.at[:, pl.ds(p * D + hf * (D // 2), D // 2)],
            wqk_v.at[n], sems.at[_SEM_QK + n])

    def v_copy():
        return pltpu.make_async_copy(
            wqkv_hbm.at[:, pl.ds(2 * D, D)], wv_v, sems.at[_SEM_V])

    def wo_copy():
        return pltpu.make_async_copy(wo_hbm, wo_v, sems.at[_SEM_WO])

    def f_copies(c):
        off = c * FC
        if not isinstance(c, int):
            off = pl.multiple_of(off, LANES)
        return [
            pltpu.make_async_copy(w1_hbm.at[:, pl.ds(off, FC)], w1_v.at[c], sems.at[_SEM_F + 3 * c]),
            pltpu.make_async_copy(w3_hbm.at[:, pl.ds(off, FC)], w3_v.at[c], sems.at[_SEM_F + 3 * c + 1]),
            pltpu.make_async_copy(w2_hbm.at[pl.ds(off, FC), :], w2_v.at[c], sems.at[_SEM_F + 3 * c + 2]),
        ]

    @pl.when(step == 0)
    def _():
        for nx in range(XCH):
            x0_copy(nx).start()
        for n in range(4):
            qk_copy(n).start()
        v_copy().start()
        for c in range(NC):
            for cp in f_copies(c):
                cp.start()
            if c == 0:
                x_copy(1).start()
            if c == 1:
                wo_copy().start()
                for t in range(2, NSTEP):
                    x_copy(t).start()
        for nx in range(XCH):
            n = TM // XCH
            x0_copy(nx).wait()
            xn_v[0, nx * n:(nx + 1) * n, :] = _layernorm(x_v[0, nx * n:(nx + 1) * n, :])
        qk_copy(0).wait()

    def qk_tile(n, i):
        return wqk_v[n, :, i * LANES:(i + 1) * LANES]

    HT = NT // 2
    first = step == 0
    for buf in (k_v, v_v):
        buf[:, 0:HALO, :] = jnp.where(first, 0.0, buf[:, TM:TM + HALO, :])
    xn = xn_v[cur]
    for i in range(HT):
        q_v[i] = jnp.dot(xn, qk_tile(0, i), preferred_element_type=_F32)

    @pl.when(step == 0)
    def _():
        qk_copy(1).wait()
        qk_copy(2).wait()

    xn = xn_v[cur]
    for i in range(HT):
        q_v[HT + i] = jnp.dot(xn, qk_tile(1, i), preferred_element_type=_F32)
    for i in range(HT):
        k_v[i, HALO:HALO + TM, :] = jnp.dot(xn, qk_tile(2, i), preferred_element_type=_F32)

    @pl.when(step == 0)
    def _():
        qk_copy(3).wait()
        v_copy().wait()

    xn = xn_v[cur]
    for i in range(HT):
        k_v[HT + i, HALO:HALO + TM, :] = jnp.dot(xn, qk_tile(3, i), preferred_element_type=_F32)
    _prep_cols(wv_v, wv_p, 0, D)
    for i in range(NT):
        v_v[i, HALO:HALO + TM, :] = jnp.dot(xn, pltpu.bitcast(wv_p[i], _BF16), preferred_element_type=_F32)

    row = jax.lax.broadcasted_iota(jnp.int32, (RB, LANES), 0)
    scale = DH ** -0.5
    lane = jax.lax.broadcasted_iota(jnp.int32, (RB, LANES), 1)
    odd1 = (lane & 1) != 0
    odd2 = (lane & 2) != 0

    def attn_block(r0):
        grow = row + (step * TM + r0)
        qs = [q_v[i, pl.ds(r0, RB), :] for i in range(NT)]
        s = []
        for i in range(NT):
            kst = jnp.concatenate(
                [k_v[i, pl.ds(r0 + HALO - DIL * w, RB), :] for w in range(W)], axis=0)
            s.append(jnp.concatenate([qs[i]] * W, axis=0) * kst)
        lane_w = jax.lax.broadcasted_iota(jnp.int32, (W * RB, LANES), 1)
        for b in range(3):
            sh = 4 << b
            lo = (lane_w & sh) == 0
            s = [jnp.where(lo, s[2 * a] + pltpu.roll(s[2 * a], LANES - sh, 1),
                           s[2 * a + 1] + pltpu.roll(s[2 * a + 1], sh, 1))
                 for a in range(len(s) // 2)]
        acc = s[0]
        acc = acc + jnp.where((lane_w & 1) != 0, pltpu.roll(acc, 1, 1), pltpu.roll(acc, LANES - 1, 1))
        acc = acc + jnp.where((lane_w & 2) != 0, pltpu.roll(acc, 2, 1), pltpu.roll(acc, LANES - 2, 1))
        acc = acc * scale
        logits = []
        for w in range(W):
            l = acc[w * RB:(w + 1) * RB, :]
            if w > 0:
                l = jnp.where(grow >= DIL * w, l, -1e9)
            logits.append(l)
        mx = logits[0]
        for w in range(1, W):
            mx = jnp.maximum(mx, logits[w])
        es = [jnp.exp(l - mx) for l in logits]
        den = es[0]
        for w in range(1, W):
            den = den + es[w]
        inv = 1.0 / den
        ps = [e * inv for e in es]
        os_ = []
        for i in range(NT):
            acc = None
            for w in range(W):
                p = ps[w] * v_v[i, pl.ds(r0 + HALO - DIL * w, RB), :]
                acc = p if acc is None else acc + p
            os_.append(acc)
        os_ = _lane_butterfly(os_)
        for i in range(NT):
            o_v[pl.ds(r0, RB), i * LANES:(i + 1) * LANES] = os_[i].astype(_BF16)

    def ffn_body(c, carry):
        @pl.when(step == 0)
        def _():
            for cp in f_copies(c):
                cp.wait()

        @pl.when(jnp.logical_and(c == 0, step < NSTEP - 1))
        def _():
            x_copy(step + 1).wait()

        base = pl.multiple_of(c * AR, AR)

        def part_f():
            xn = xn_v[cur]
            gate = jnp.dot(xn, w1_v[c], preferred_element_type=_F32)
            up = jnp.dot(xn, w3_v[c], preferred_element_type=_F32)
            h = (gate * jax.nn.sigmoid(gate) * up).astype(_BF16)
            d = jnp.dot(h, w2_v[c], preferred_element_type=_F32)
            acc_v[...] = jnp.where(c > 0, acc_v[...], 0.0) + d

        def part_a():
            for b in range(AR // RB):
                attn_block(base + b * RB)

        def part_l():
            nt = jnp.minimum(step + 1, NSTEP - 1)
            xn_v[nxt, pl.ds(base, AR), :] = _layernorm(x_v[nt, pl.ds(base, AR), :])

        for ch in "FAL":
            {"F": part_f, "A": part_a, "L": part_l}[ch]()
        return carry

    jax.lax.fori_loop(0, NC, ffn_body, 0)

    @pl.when(step == 0)
    def _():
        wo_copy().wait()

    OC = D // OCH

    def out_copy(t, ch):
        return pltpu.make_async_copy(
            out_v.at[ch], out_hbm.at[pl.ds(t * TM, TM), pl.ds(ch * OC, OC)],
            sems.at[_SEM_OUT + ch])

    @pl.when(step > 0)
    def _():
        for ch in range(OCH):
            out_copy(step - 1, ch).wait()

    o = o_v[...]
    for ct in range(NT):
        cols = slice(ct * LANES, (ct + 1) * LANES)
        s = jnp.dot(o, wo_v[:, cols], preferred_element_type=_F32)
        ffn = acc_v[:, cols]
        g = ffn * jax.nn.sigmoid(ffn)
        per = NT // OCH
        ch, sub = ct // per, ct % per
        out_v[ch, :, sub * LANES:(sub + 1) * LANES] = (
            x_v[step, :, cols].astype(_F32) + s * g).astype(out_v.dtype)
        if sub == per - 1:
            out_copy(step, ch).start()

    @pl.when(step == NSTEP - 1)
    def _():
        for ch in range(OCH):
            out_copy(step, ch).wait()


@jax.jit
def pallas_recurrent_scan__sliding_local_dilated__glu_gated_swiglu__prompt_kernel(
    A_x: jax.Array,
    A_wqkv: jax.Array,
    A_wo: jax.Array,
    B_x: jax.Array,
    B_w1: jax.Array,
    B_w3: jax.Array,
    B_w2: jax.Array,
):
    x = A_x.reshape(S, D)
    any_spec = pl.BlockSpec(memory_space=pl.ANY)
    wp = pltpu.VMEM((NT, D // 2, LANES), _U32)
    out = pl.pallas_call(
        _kernel,
        grid=(NSTEP,),
        in_specs=[any_spec] * 6,
        out_specs=any_spec,
        out_shape=jax.ShapeDtypeStruct((S, D), A_x.dtype),
        scratch_shapes=[
            pltpu.VMEM((NSTEP, TM, D), _BF16),
            pltpu.VMEM((4, D, D // 2), _BF16),
            pltpu.VMEM((D, D), _BF16),
            pltpu.VMEM((D, D), _BF16),
            pltpu.VMEM((NC, D, FC), _BF16),
            pltpu.VMEM((NC, D, FC), _BF16),
            pltpu.VMEM((NC, FC, D), _BF16),
            wp,
            pltpu.VMEM((2, TM, D), _BF16),
            pltpu.VMEM((NT, TM, LANES), _F32),
            pltpu.VMEM((NT, TM + HALO, LANES), _F32),
            pltpu.VMEM((NT, TM + HALO, LANES), _F32),
            pltpu.VMEM((TM, D), _BF16),
            pltpu.VMEM((TM, D), _F32),
            pltpu.VMEM((OCH, TM, D // OCH), _BF16),
            pltpu.SemaphoreType.DMA((_NSEM,)),
        ],
        compiler_params=pltpu.CompilerParams(
            dimension_semantics=("arbitrary",),
            vmem_limit_bytes=110 * 1024 * 1024,
        ),
        name="fused_block",
    )(x, A_wqkv, A_wo, B_w1, B_w3, B_w2)
    return out.reshape(A_x.shape)
```

```python
import functools

import jax
import jax.numpy as jnp
import jax.experimental.pallas as pl
import jax.experimental.pallas.tpu as pltpu

S = 2048
D = 1024
H = 32
DH = 32
W = 8
DIL = 2
F = 3584
LANES = 128
NT = D // LANES
HALO = 16

TM = 512
NSTEP = S // TM
FC = 896
NC = F // FC
RB = 8
AR = TM // NC
QCH = 8
OCH = 8
PERMS = 'rd'
XCH = 4
PR = 128

_F32 = jnp.float32
_BF16 = jnp.bfloat16
_U32 = jnp.uint32


def _xor_lanes(x, k):
    lane = jax.lax.broadcasted_iota(jnp.int32, x.shape, 1)
    return jnp.take_along_axis(x, lane ^ k, axis=1)


def _lane_butterfly(tiles, use_perm=False):
    s = list(tiles)
    lane = jax.lax.broadcasted_iota(jnp.int32, s[0].shape, 1)
    for b in range(3):
        sh = 4 << b
        lo = (lane & sh) == 0
        ns = list(s)
        for a in range(NT):
            if a & (1 << b):
                continue
            c = a | (1 << b)
            if use_perm:
                r = _xor_lanes(jnp.where(lo, s[c], s[a]), sh)
                ns[a] = jnp.where(lo, s[a], r)
                ns[c] = jnp.where(lo, r, s[c])
            else:
                ns[a] = jnp.where(lo, s[a], pltpu.roll(s[c], sh, 1))
                ns[c] = jnp.where(lo, pltpu.roll(s[a], LANES - sh, 1), s[c])
        s = ns
    return s


def _prep_cols(src, dst, r0, nrows, use_perm=False):
    for r in range(r0, r0 + nrows, PR):
        outs = _lane_butterfly([pltpu.bitcast(src[r:r + PR, j * LANES:(j + 1) * LANES], _U32)
                                for j in range(NT)], use_perm)
        for i in range(NT):
            dst[i, r // 2:(r + PR) // 2, :] = outs[i]


def _layernorm(xb):
    x = xb.astype(_F32)
    mu = jnp.mean(x, axis=-1, keepdims=True)
    xc = x - mu
    var = jnp.mean(xc * xc, axis=-1, keepdims=True)
    return (xc * jax.lax.rsqrt(var + 1e-5)).astype(_BF16)


_SEM_X = 0
_SEM_X0 = _SEM_X + NSTEP
_SEM_QK = _SEM_X0 + XCH
_SEM_V = _SEM_QK + 4
_SEM_WO = _SEM_V + 1
_SEM_F = _SEM_WO + 1
_SEM_OUT = _SEM_F + 3 * NC
_NSEM = _SEM_OUT + OCH


def _kernel(x_hbm, wqkv_hbm, wo_hbm, w1_hbm, w3_hbm, w2_hbm, out_hbm,
            x_v, wqk_v, wv_v, wo_v, w1_v, w3_v, w2_v, wv_p,
            xn_v, q_v, k_v, v_v, o_v, acc_v, out_v, sems):
    step = pl.program_id(0)
    cur = step % 2
    nxt = 1 - cur
    QR = D // QCH

    def x_copy(t):
        return pltpu.make_async_copy(
            x_hbm.at[pl.ds(t * TM, TM), :], x_v.at[t], sems.at[_SEM_X + t])

    def x0_copy(ch):
        n = TM // XCH
        return pltpu.make_async_copy(
            x_hbm.at[pl.ds(ch * n, n), :], x_v.at[0, pl.ds(ch * n, n), :], sems.at[_SEM_X0 + ch])

    def qk_copy(n):
        p, hf = n // 2, n % 2
        return pltpu.make_async_copy(
            wqkv_hbm.at[:, pl.ds(p * D + hf * (D // 2), D // 2)],
            wqk_v.at[n], sems.at[_SEM_QK + n])

    def v_copy():
        return pltpu.make_async_copy(
            wqkv_hbm.at[:, pl.ds(2 * D, D)], wv_v, sems.at[_SEM_V])

    def wo_copy():
        return pltpu.make_async_copy(wo_hbm, wo_v, sems.at[_SEM_WO])

    def f_copies(c):
        off = c * FC
        if not isinstance(c, int):
            off = pl.multiple_of(off, LANES)
        return [
            pltpu.make_async_copy(w1_hbm.at[:, pl.ds(off, FC)], w1_v.at[c], sems.at[_SEM_F + 3 * c]),
            pltpu.make_async_copy(w3_hbm.at[:, pl.ds(off, FC)], w3_v.at[c], sems.at[_SEM_F + 3 * c + 1]),
            pltpu.make_async_copy(w2_hbm.at[pl.ds(off, FC), :], w2_v.at[c], sems.at[_SEM_F + 3 * c + 2]),
        ]

    @pl.when(step == 0)
    def _():
        for nx in range(XCH):
            x0_copy(nx).start()
        for n in range(4):
            qk_copy(n).start()
        v_copy().start()
        for c in range(NC):
            for cp in f_copies(c):
                cp.start()
            if c == 0:
                x_copy(1).start()
            if c == 1:
                wo_copy().start()
                for t in range(2, NSTEP):
                    x_copy(t).start()
        for nx in range(XCH):
            n = TM // XCH
            x0_copy(nx).wait()
            xn_v[0, nx * n:(nx + 1) * n, :] = _layernorm(x_v[0, nx * n:(nx + 1) * n, :])
        qk_copy(0).wait()

    def qk_tile(n, i):
        return wqk_v[n, :, i * LANES:(i + 1) * LANES]

    HT = NT // 2
    def block1(first):
        for buf in (k_v, v_v):
            if first:
                buf[:, 0:HALO, :] = jnp.zeros((NT, HALO, LANES), _F32)
            else:
                buf[:, 0:HALO, :] = buf[:, TM:TM + HALO, :]
        xn = xn_v[cur]
        for i in range(HT):
            q_v[i] = jnp.dot(xn, qk_tile(0, i), preferred_element_type=_F32)

    def block2():
        xn = xn_v[cur]
        for i in range(HT):
            q_v[HT + i] = jnp.dot(xn, qk_tile(1, i), preferred_element_type=_F32)
        for i in range(HT):
            k_v[i, HALO:HALO + TM, :] = jnp.dot(xn, qk_tile(2, i), preferred_element_type=_F32)

    @pl.when(step == 0)
    def _():
        block1(True)
        qk_copy(1).wait()
        qk_copy(2).wait()
        block2()

    @pl.when(step > 0)
    def _():
        block1(False)
        block2()

    @pl.when(step == 0)
    def _():
        qk_copy(3).wait()
        v_copy().wait()

    xn = xn_v[cur]
    for i in range(HT):
        k_v[HT + i, HALO:HALO + TM, :] = jnp.dot(xn, qk_tile(3, i), preferred_element_type=_F32)
    _prep_cols(wv_v, wv_p, 0, D)
    for i in range(NT):
        v_v[i, HALO:HALO + TM, :] = jnp.dot(xn, pltpu.bitcast(wv_p[i], _BF16), preferred_element_type=_F32)

    row = jax.lax.broadcasted_iota(jnp.int32, (RB, LANES), 0)
    scale = DH ** -0.5
    lane = jax.lax.broadcasted_iota(jnp.int32, (RB, LANES), 1)
    odd1 = (lane & 1) != 0
    odd2 = (lane & 2) != 0

    def attn_block(r0):
        grow = row + (step * TM + r0)
        qs = [q_v[i, pl.ds(r0, RB), :] for i in range(NT)]
        s = []
        for i in range(NT):
            kst = jnp.concatenate(
                [k_v[i, pl.ds(r0 + HALO - DIL * w, RB), :] for w in range(W)], axis=0)
            s.append(jnp.concatenate([qs[i]] * W, axis=0) * kst)
        lane_w = jax.lax.broadcasted_iota(jnp.int32, (W * RB, LANES), 1)
        for b in range(3):
            sh = 4 << b
            lo = (lane_w & sh) == 0
            if "r" in PERMS:
                s = [jnp.where(lo, s[2 * a], s[2 * a + 1])
                     + _xor_lanes(jnp.where(lo, s[2 * a + 1], s[2 * a]), sh)
                     for a in range(len(s) // 2)]
            else:
                s = [jnp.where(lo, s[2 * a] + pltpu.roll(s[2 * a], LANES - sh, 1),
                               s[2 * a + 1] + pltpu.roll(s[2 * a + 1], sh, 1))
                     for a in range(len(s) // 2)]
        acc = s[0]
        if "d" in PERMS:
            acc = acc + _xor_lanes(acc, 1)
            acc = acc + _xor_lanes(acc, 2)
        else:
            acc = acc + jnp.where((lane_w & 1) != 0, pltpu.roll(acc, 1, 1), pltpu.roll(acc, LANES - 1, 1))
            acc = acc + jnp.where((lane_w & 2) != 0, pltpu.roll(acc, 2, 1), pltpu.roll(acc, LANES - 2, 1))
        acc = acc * scale
        logits = []
        for w in range(W):
            l = acc[w * RB:(w + 1) * RB, :]
            if w > 0:
                l = jnp.where(grow >= DIL * w, l, -1e9)
            logits.append(l)
        mx = logits[0]
        for w in range(1, W):
            mx = jnp.maximum(mx, logits[w])
        es = [jnp.exp(l - mx) for l in logits]
        den = es[0]
        for w in range(1, W):
            den = den + es[w]
        inv = 1.0 / den
        ps = [e * inv for e in es]
        os_ = []
        for i in range(NT):
            acc = None
            for w in range(W):
                p = ps[w] * v_v[i, pl.ds(r0 + HALO - DIL * w, RB), :]
                acc = p if acc is None else acc + p
            os_.append(acc)
        os_ = _lane_butterfly(os_, "o" in PERMS)
        for i in range(NT):
            o_v[pl.ds(r0, RB), i * LANES:(i + 1) * LANES] = os_[i].astype(_BF16)

    def ffn_body(c, carry):
        @pl.when(step == 0)
        def _():
            for cp in f_copies(c):
                cp.wait()

        @pl.when(jnp.logical_and(c == 0, step < NSTEP - 1))
        def _():
            x_copy(step + 1).wait()

        base = pl.multiple_of(c * AR, AR)

        def part_f():
            xn = xn_v[cur]
            gate = jnp.dot(xn, w1_v[c], preferred_element_type=_F32)
            up = jnp.dot(xn, w3_v[c], preferred_element_type=_F32)
            h = (gate * jax.nn.sigmoid(gate) * up).astype(_BF16)
            d = jnp.dot(h, w2_v[c], preferred_element_type=_F32)
            acc_v[...] = jnp.where(c > 0, acc_v[...], 0.0) + d

        def part_a():
            for b in range(AR // RB):
                attn_block(base + b * RB)

        def part_l():
            nt = jnp.minimum(step + 1, NSTEP - 1)
            xn_v[nxt, pl.ds(base, AR), :] = _layernorm(x_v[nt, pl.ds(base, AR), :])

        for ch in "FAL":
            {"F": part_f, "A": part_a, "L": part_l}[ch]()
        return carry

    jax.lax.fori_loop(0, NC, ffn_body, 0)

    @pl.when(step == 0)
    def _():
        wo_copy().wait()

    OC = D // OCH

    def out_copy(t, ch):
        return pltpu.make_async_copy(
            out_v.at[ch], out_hbm.at[pl.ds(t * TM, TM), pl.ds(ch * OC, OC)],
            sems.at[_SEM_OUT + ch])

    @pl.when(step > 0)
    def _():
        for ch in range(OCH):
            out_copy(step - 1, ch).wait()

    o = o_v[...]
    for ct in range(NT):
        cols = slice(ct * LANES, (ct + 1) * LANES)
        s = jnp.dot(o, wo_v[:, cols], preferred_element_type=_F32)
        ffn = acc_v[:, cols]
        g = ffn * jax.nn.sigmoid(ffn)
        per = NT // OCH
        ch, sub = ct // per, ct % per
        out_v[ch, :, sub * LANES:(sub + 1) * LANES] = (
            x_v[step, :, cols].astype(_F32) + s * g).astype(out_v.dtype)
        if sub == per - 1:
            out_copy(step, ch).start()

    @pl.when(step == NSTEP - 1)
    def _():
        for ch in range(OCH):
            out_copy(step, ch).wait()


@jax.jit
def pallas_recurrent_scan__sliding_local_dilated__glu_gated_swiglu__prompt_kernel(
    A_x: jax.Array,
    A_wqkv: jax.Array,
    A_wo: jax.Array,
    B_x: jax.Array,
    B_w1: jax.Array,
    B_w3: jax.Array,
    B_w2: jax.Array,
):
    x = A_x.reshape(S, D)
    any_spec = pl.BlockSpec(memory_space=pl.ANY)
    wp = pltpu.VMEM((NT, D // 2, LANES), _U32)
    out = pl.pallas_call(
        _kernel,
        grid=(NSTEP,),
        in_specs=[any_spec] * 6,
        out_specs=any_spec,
        out_shape=jax.ShapeDtypeStruct((S, D), A_x.dtype),
        scratch_shapes=[
            pltpu.VMEM((NSTEP, TM, D), _BF16),
            pltpu.VMEM((4, D, D // 2), _BF16),
            pltpu.VMEM((D, D), _BF16),
            pltpu.VMEM((D, D), _BF16),
            pltpu.VMEM((NC, D, FC), _BF16),
            pltpu.VMEM((NC, D, FC), _BF16),
            pltpu.VMEM((NC, FC, D), _BF16),
            wp,
            pltpu.VMEM((2, TM, D), _BF16),
            pltpu.VMEM((NT, TM, LANES), _F32),
            pltpu.VMEM((NT, TM + HALO, LANES), _F32),
            pltpu.VMEM((NT, TM + HALO, LANES), _F32),
            pltpu.VMEM((TM, D), _BF16),
            pltpu.VMEM((TM, D), _F32),
            pltpu.VMEM((OCH, TM, D // OCH), _BF16),
            pltpu.SemaphoreType.DMA((_NSEM,)),
        ],
        compiler_params=pltpu.CompilerParams(
            dimension_semantics=("arbitrary",),
            vmem_limit_bytes=110 * 1024 * 1024,
        ),
        name="fused_block",
    )(x, A_wqkv, A_wo, B_w1, B_w3, B_w2)
    return out.reshape(A_x.shape)
```

```python
import functools

import jax
import jax.numpy as jnp
import jax.experimental.pallas as pl
import jax.experimental.pallas.tpu as pltpu

S = 2048
D = 1024
H = 32
DH = 32
W = 8
DIL = 2
F = 3584
LANES = 128
NT = D // LANES
HALO = 16

TM = 512
NSTEP = S // TM
FC = 896
NC = F // FC
RB = 8
AR = TM // NC
QCH = 8
OCH = 8
PERMS = 'rd'
XCH = 4
PR = 128

_F32 = jnp.float32
_BF16 = jnp.bfloat16
_U32 = jnp.uint32


def _xor_lanes(x, k):
    lane = jax.lax.broadcasted_iota(jnp.int32, x.shape, 1)
    return jnp.take_along_axis(x, lane ^ k, axis=1)


def _lane_butterfly(tiles, use_perm=False):
    s = list(tiles)
    lane = jax.lax.broadcasted_iota(jnp.int32, s[0].shape, 1)
    for b in range(3):
        sh = 4 << b
        lo = (lane & sh) == 0
        ns = list(s)
        for a in range(NT):
            if a & (1 << b):
                continue
            c = a | (1 << b)
            if use_perm:
                r = _xor_lanes(jnp.where(lo, s[c], s[a]), sh)
                ns[a] = jnp.where(lo, s[a], r)
                ns[c] = jnp.where(lo, r, s[c])
            else:
                ns[a] = jnp.where(lo, s[a], pltpu.roll(s[c], sh, 1))
                ns[c] = jnp.where(lo, pltpu.roll(s[a], LANES - sh, 1), s[c])
        s = ns
    return s


def _prep_cols(src, dst, r0, nrows, use_perm=False):
    for r in range(r0, r0 + nrows, PR):
        outs = _lane_butterfly([pltpu.bitcast(src[r:r + PR, j * LANES:(j + 1) * LANES], _U32)
                                for j in range(NT)], use_perm)
        for i in range(NT):
            dst[i, r // 2:(r + PR) // 2, :] = outs[i]


def _layernorm(xb):
    x = xb.astype(_F32)
    mu = jnp.mean(x, axis=-1, keepdims=True)
    xc = x - mu
    var = jnp.mean(xc * xc, axis=-1, keepdims=True)
    return (xc * jax.lax.rsqrt(var + 1e-5)).astype(_BF16)


_SEM_X = 0
_SEM_X0 = _SEM_X + NSTEP
_SEM_QK = _SEM_X0 + XCH
_SEM_V = _SEM_QK + 4
_SEM_WO = _SEM_V + 1
_SEM_F = _SEM_WO + 1
_SEM_OUT = _SEM_F + 3 * NC
_NSEM = _SEM_OUT + OCH


def _kernel(x_hbm, wqkv_hbm, wo_hbm, w1_hbm, w3_hbm, w2_hbm, out_hbm,
            x_v, wqk_v, wv_v, wo_v, w1_v, w3_v, w2_v, wv_p,
            xn_v, qk_v, v_v, o_v, acc_v, out_v, sems):
    step = pl.program_id(0)
    cur = step % 2
    nxt = 1 - cur
    QR = D // QCH

    def x_copy(t):
        return pltpu.make_async_copy(
            x_hbm.at[pl.ds(t * TM, TM), :], x_v.at[t], sems.at[_SEM_X + t])

    def x0_copy(ch):
        n = TM // XCH
        return pltpu.make_async_copy(
            x_hbm.at[pl.ds(ch * n, n), :], x_v.at[0, pl.ds(ch * n, n), :], sems.at[_SEM_X0 + ch])

    def qk_copy(n):
        off = n * (D // 2)
        if not isinstance(n, int):
            off = pl.multiple_of(off, D // 2)
        return pltpu.make_async_copy(
            wqkv_hbm.at[:, pl.ds(off, D // 2)],
            wqk_v.at[n], sems.at[_SEM_QK + n])

    def v_copy():
        return pltpu.make_async_copy(
            wqkv_hbm.at[:, pl.ds(2 * D, D)], wv_v, sems.at[_SEM_V])

    def wo_copy():
        return pltpu.make_async_copy(wo_hbm, wo_v, sems.at[_SEM_WO])

    def f_copies(c):
        off = c * FC
        if not isinstance(c, int):
            off = pl.multiple_of(off, LANES)
        return [
            pltpu.make_async_copy(w1_hbm.at[:, pl.ds(off, FC)], w1_v.at[c], sems.at[_SEM_F + 3 * c]),
            pltpu.make_async_copy(w3_hbm.at[:, pl.ds(off, FC)], w3_v.at[c], sems.at[_SEM_F + 3 * c + 1]),
            pltpu.make_async_copy(w2_hbm.at[pl.ds(off, FC), :], w2_v.at[c], sems.at[_SEM_F + 3 * c + 2]),
        ]

    @pl.when(step == 0)
    def _():
        for nx in range(XCH):
            x0_copy(nx).start()
        for n in range(4):
            qk_copy(n).start()
        v_copy().start()
        for c in range(NC):
            for cp in f_copies(c):
                cp.start()
            if c == 0:
                x_copy(1).start()
            if c == 1:
                wo_copy().start()
                for t in range(2, NSTEP):
                    x_copy(t).start()
        for nx in range(XCH):
            n = TM // XCH
            x0_copy(nx).wait()
            xn_v[0, nx * n:(nx + 1) * n, :] = _layernorm(x_v[0, nx * n:(nx + 1) * n, :])

    def qk_tile(n, i):
        return wqk_v[n, :, i * LANES:(i + 1) * LANES]

    HT = NT // 2

    def halo(first):
        for buf, lo in ((qk_v, NT), (v_v, 0)):
            if first:
                buf[lo:lo + NT, 0:HALO, :] = jnp.zeros((NT, HALO, LANES), _F32)
            else:
                buf[lo:lo + NT, 0:HALO, :] = buf[lo:lo + NT, TM:TM + HALO, :]

    def block12(slot):
        xn = xn_v[slot]
        for g in range(3):
            for i in range(HT):
                qk_v[HT * g + i, HALO:HALO + TM, :] = jnp.dot(
                    xn, qk_tile(g, i), preferred_element_type=_F32)

    @pl.when(step == 0)
    def _():
        halo(True)

        def group(g, carry):
            qk_copy(g).wait()
            xn = xn_v[0]
            for i in range(HT):
                qk_v[HT * g + i, HALO:HALO + TM, :] = jnp.dot(
                    xn, qk_tile(g, i), preferred_element_type=_F32)
            return carry

        jax.lax.fori_loop(0, 3, group, 0)

    @pl.when(step == 0)
    def _():
        qk_copy(3).wait()
        v_copy().wait()

    xn = xn_v[cur]
    for i in range(HT):
        qk_v[NT + HT + i, HALO:HALO + TM, :] = jnp.dot(xn, qk_tile(3, i), preferred_element_type=_F32)
    _prep_cols(wv_v, wv_p, 0, D, "0" == "1")
    for i in range(NT):
        v_v[i, HALO:HALO + TM, :] = jnp.dot(xn, pltpu.bitcast(wv_p[i], _BF16), preferred_element_type=_F32)

    row = jax.lax.broadcasted_iota(jnp.int32, (RB, LANES), 0)
    scale = DH ** -0.5
    lane = jax.lax.broadcasted_iota(jnp.int32, (RB, LANES), 1)
    odd1 = (lane & 1) != 0
    odd2 = (lane & 2) != 0

    def attn_block(r0):
        grow = row + (step * TM + r0)
        qs = [qk_v[i, pl.ds(r0 + HALO, RB), :] for i in range(NT)]
        s = []
        for i in range(NT):
            kst = jnp.concatenate(
                [qk_v[NT + i, pl.ds(r0 + HALO - DIL * w, RB), :] for w in range(W)], axis=0)
            s.append(jnp.concatenate([qs[i]] * W, axis=0) * kst)
        lane_w = jax.lax.broadcasted_iota(jnp.int32, (W * RB, LANES), 1)
        for b in range(3):
            sh = 4 << b
            lo = (lane_w & sh) == 0
            if "r" in PERMS:
                s = [jnp.where(lo, s[2 * a], s[2 * a + 1])
                     + _xor_lanes(jnp.where(lo, s[2 * a + 1], s[2 * a]), sh)
                     for a in range(len(s) // 2)]
            else:
                s = [jnp.where(lo, s[2 * a] + pltpu.roll(s[2 * a], LANES - sh, 1),
                               s[2 * a + 1] + pltpu.roll(s[2 * a + 1], sh, 1))
                     for a in range(len(s) // 2)]
        acc = s[0]
        if "d" in PERMS:
            acc = acc + _xor_lanes(acc, 1)
            acc = acc + _xor_lanes(acc, 2)
        else:
            acc = acc + jnp.where((lane_w & 1) != 0, pltpu.roll(acc, 1, 1), pltpu.roll(acc, LANES - 1, 1))
            acc = acc + jnp.where((lane_w & 2) != 0, pltpu.roll(acc, 2, 1), pltpu.roll(acc, LANES - 2, 1))
        acc = acc * scale
        logits = []
        for w in range(W):
            l = acc[w * RB:(w + 1) * RB, :]
            if w > 0:
                l = jnp.where(grow >= DIL * w, l, -1e9)
            logits.append(l)
        mx = logits[0]
        for w in range(1, W):
            mx = jnp.maximum(mx, logits[w])
        es = [jnp.exp(l - mx) for l in logits]
        den = es[0]
        for w in range(1, W):
            den = den + es[w]
        inv = 1.0 / den
        ps = [e * inv for e in es]
        os_ = []
        for i in range(NT):
            acc = None
            for w in range(W):
                p = ps[w] * v_v[i, pl.ds(r0 + HALO - DIL * w, RB), :]
                acc = p if acc is None else acc + p
            os_.append(acc)
        os_ = _lane_butterfly(os_, "o" in PERMS)
        for i in range(NT):
            o_v[pl.ds(r0, RB), i * LANES:(i + 1) * LANES] = os_[i].astype(_BF16)

    def ffn_body(c, carry):
        @pl.when(step == 0)
        def _():
            for cp in f_copies(c):
                cp.wait()

        @pl.when(jnp.logical_and(c == 0, step < NSTEP - 1))
        def _():
            x_copy(step + 1).wait()

        base = pl.multiple_of(c * AR, AR)

        def part_f():
            xn = xn_v[cur]
            gate = jnp.dot(xn, w1_v[c], preferred_element_type=_F32)
            up = jnp.dot(xn, w3_v[c], preferred_element_type=_F32)
            h = (gate * jax.nn.sigmoid(gate) * up).astype(_BF16)
            d = jnp.dot(h, w2_v[c], preferred_element_type=_F32)
            acc_v[...] = jnp.where(c > 0, acc_v[...], 0.0) + d

        def part_a():
            for b in range(AR // RB):
                attn_block(base + b * RB)

        def part_l():
            nt = jnp.minimum(step + 1, NSTEP - 1)
            xn_v[nxt, pl.ds(base, AR), :] = _layernorm(x_v[nt, pl.ds(base, AR), :])

        for ch in "FAL":
            {"F": part_f, "A": part_a, "L": part_l}[ch]()
        return carry

    jax.lax.fori_loop(0, NC, ffn_body, 0)

    @pl.when(step == 0)
    def _():
        wo_copy().wait()

    OC = D // OCH

    def out_copy(t, ch):
        return pltpu.make_async_copy(
            out_v.at[ch], out_hbm.at[pl.ds(t * TM, TM), pl.ds(ch * OC, OC)],
            sems.at[_SEM_OUT + ch])

    @pl.when(step > 0)
    def _():
        for ch in range(OCH):
            out_copy(step - 1, ch).wait()

    def out_block():
        o = o_v[...]
        for ct in range(NT):
            cols = slice(ct * LANES, (ct + 1) * LANES)
            s = jnp.dot(o, wo_v[:, cols], preferred_element_type=_F32)
            ffn = acc_v[:, cols]
            g = ffn * jax.nn.sigmoid(ffn)
            per = NT // OCH
            ch, sub = ct // per, ct % per
            out_v[ch, :, sub * LANES:(sub + 1) * LANES] = (
                x_v[step, :, cols].astype(_F32) + s * g).astype(out_v.dtype)
            if sub == per - 1:
                out_copy(step, ch).start()

    @pl.when(step < NSTEP - 1)
    def _():
        out_block()
        halo(False)
        block12(nxt)

    @pl.when(step == NSTEP - 1)
    def _():
        out_block()

    @pl.when(step == NSTEP - 1)
    def _():
        for ch in range(OCH):
            out_copy(step, ch).wait()


@jax.jit
def pallas_recurrent_scan__sliding_local_dilated__glu_gated_swiglu__prompt_kernel(
    A_x: jax.Array,
    A_wqkv: jax.Array,
    A_wo: jax.Array,
    B_x: jax.Array,
    B_w1: jax.Array,
    B_w3: jax.Array,
    B_w2: jax.Array,
):
    x = A_x.reshape(S, D)
    any_spec = pl.BlockSpec(memory_space=pl.ANY)
    wp = pltpu.VMEM((NT, D // 2, LANES), _U32)
    out = pl.pallas_call(
        _kernel,
        grid=(NSTEP,),
        in_specs=[any_spec] * 6,
        out_specs=any_spec,
        out_shape=jax.ShapeDtypeStruct((S, D), A_x.dtype),
        scratch_shapes=[
            pltpu.VMEM((NSTEP, TM, D), _BF16),
            pltpu.VMEM((4, D, D // 2), _BF16),
            pltpu.VMEM((D, D), _BF16),
            pltpu.VMEM((D, D), _BF16),
            pltpu.VMEM((NC, D, FC), _BF16),
            pltpu.VMEM((NC, D, FC), _BF16),
            pltpu.VMEM((NC, FC, D), _BF16),
            wp,
            pltpu.VMEM((2, TM, D), _BF16),
            pltpu.VMEM((2 * NT, TM + HALO, LANES), _F32),
            pltpu.VMEM((NT, TM + HALO, LANES), _F32),
            pltpu.VMEM((TM, D), _BF16),
            pltpu.VMEM((TM, D), _F32),
            pltpu.VMEM((OCH, TM, D // OCH), _BF16),
            pltpu.SemaphoreType.DMA((_NSEM,)),
        ],
        compiler_params=pltpu.CompilerParams(
            dimension_semantics=("arbitrary",),
            vmem_limit_bytes=110 * 1024 * 1024,
        ),
        name="fused_block",
    )(x, A_wqkv, A_wo, B_w1, B_w3, B_w2)
    return out.reshape(A_x.shape)
```

```python
import functools

import jax
import jax.numpy as jnp
import jax.experimental.pallas as pl
import jax.experimental.pallas.tpu as pltpu

S = 2048
D = 1024
H = 32
DH = 32
W = 8
DIL = 2
F = 3584
LANES = 128
NT = D // LANES
HALO = 16

TM = 512
NSTEP = S // TM
FC = 896
NC = F // FC
RB = 8
AR = TM // NC
QCH = 8
OCH = 8
PERMS = 'rd'
GT = 2
NG = 12 // GT
XCH = 4
PR = 128

_F32 = jnp.float32
_BF16 = jnp.bfloat16
_U32 = jnp.uint32


def _xor_lanes(x, k):
    lane = jax.lax.broadcasted_iota(jnp.int32, x.shape, 1)
    return jnp.take_along_axis(x, lane ^ k, axis=1)


def _lane_butterfly(tiles, use_perm=False):
    s = list(tiles)
    lane = jax.lax.broadcasted_iota(jnp.int32, s[0].shape, 1)
    for b in range(3):
        sh = 4 << b
        lo = (lane & sh) == 0
        ns = list(s)
        for a in range(NT):
            if a & (1 << b):
                continue
            c = a | (1 << b)
            if use_perm:
                r = _xor_lanes(jnp.where(lo, s[c], s[a]), sh)
                ns[a] = jnp.where(lo, s[a], r)
                ns[c] = jnp.where(lo, r, s[c])
            else:
                ns[a] = jnp.where(lo, s[a], pltpu.roll(s[c], sh, 1))
                ns[c] = jnp.where(lo, pltpu.roll(s[a], LANES - sh, 1), s[c])
        s = ns
    return s


def _prep_cols(src, dst, r0, nrows, use_perm=False):
    for r in range(r0, r0 + nrows, PR):
        outs = _lane_butterfly([pltpu.bitcast(src[r:r + PR, j * LANES:(j + 1) * LANES], _U32)
                                for j in range(NT)], use_perm)
        for i in range(NT):
            dst[i, r // 2:(r + PR) // 2, :] = outs[i]


def _layernorm(xb):
    x = xb.astype(_F32)
    mu = jnp.mean(x, axis=-1, keepdims=True)
    xc = x - mu
    var = jnp.mean(xc * xc, axis=-1, keepdims=True)
    return (xc * jax.lax.rsqrt(var + 1e-5)).astype(_BF16)


_SEM_X = 0
_SEM_X0 = _SEM_X + NSTEP
_SEM_QK = _SEM_X0 + XCH
_SEM_V = _SEM_QK + 16 // GT
_SEM_WO = _SEM_V + 1
_SEM_F = _SEM_WO + 1
_SEM_OUT = _SEM_F + 3 * NC
_NSEM = _SEM_OUT + OCH


def _kernel(x_hbm, wqkv_hbm, wo_hbm, w1_hbm, w3_hbm, w2_hbm, out_hbm,
            x_v, wqk_v, wv_v, wo_v, w1_v, w3_v, w2_v, wv_p,
            xn_v, qk_v, v_v, o_v, acc_v, out_v, sems):
    step = pl.program_id(0)
    cur = step % 2
    nxt = 1 - cur
    QR = D // QCH

    def x_copy(t):
        return pltpu.make_async_copy(
            x_hbm.at[pl.ds(t * TM, TM), :], x_v.at[t], sems.at[_SEM_X + t])

    def x0_copy(ch):
        n = TM // XCH
        return pltpu.make_async_copy(
            x_hbm.at[pl.ds(ch * n, n), :], x_v.at[0, pl.ds(ch * n, n), :], sems.at[_SEM_X0 + ch])

    def qk_copy(n):
        off = n * (GT * LANES)
        if not isinstance(n, int):
            off = pl.multiple_of(off, LANES)
        return pltpu.make_async_copy(
            wqkv_hbm.at[:, pl.ds(off, GT * LANES)],
            wqk_v.at[n], sems.at[_SEM_QK + n])

    def v_copy():
        return pltpu.make_async_copy(
            wqkv_hbm.at[:, pl.ds(2 * D, D)], wv_v, sems.at[_SEM_V])

    def wo_copy():
        return pltpu.make_async_copy(wo_hbm, wo_v, sems.at[_SEM_WO])

    def f_copies(c):
        off = c * FC
        if not isinstance(c, int):
            off = pl.multiple_of(off, LANES)
        return [
            pltpu.make_async_copy(w1_hbm.at[:, pl.ds(off, FC)], w1_v.at[c], sems.at[_SEM_F + 3 * c]),
            pltpu.make_async_copy(w3_hbm.at[:, pl.ds(off, FC)], w3_v.at[c], sems.at[_SEM_F + 3 * c + 1]),
            pltpu.make_async_copy(w2_hbm.at[pl.ds(off, FC), :], w2_v.at[c], sems.at[_SEM_F + 3 * c + 2]),
        ]

    @pl.when(step == 0)
    def _():
        for nx in range(XCH):
            x0_copy(nx).start()
        for n in range(16 // GT):
            qk_copy(n).start()
        v_copy().start()
        for c in range(NC):
            for cp in f_copies(c):
                cp.start()
            if c == 0:
                x_copy(1).start()
            if c == 1:
                wo_copy().start()
                for t in range(2, NSTEP):
                    x_copy(t).start()
        for nx in range(XCH):
            n = TM // XCH
            x0_copy(nx).wait()
            xn_v[0, nx * n:(nx + 1) * n, :] = _layernorm(x_v[0, nx * n:(nx + 1) * n, :])

    def qk_tile(t):
        return wqk_v[t // GT, :, (t % GT) * LANES:(t % GT + 1) * LANES]

    HT = NT // 2

    def halo(first):
        for buf, lo in ((qk_v, NT), (v_v, 0)):
            if first:
                buf[lo:lo + NT, 0:HALO, :] = jnp.zeros((NT, HALO, LANES), _F32)
            else:
                buf[lo:lo + NT, 0:HALO, :] = buf[lo:lo + NT, TM:TM + HALO, :]

    def block12(slot):
        xn = xn_v[slot]
        for t in range(12):
            qk_v[t, HALO:HALO + TM, :] = jnp.dot(xn, qk_tile(t), preferred_element_type=_F32)

    @pl.when(step == 0)
    def _():
        halo(True)

        def group(g, carry):
            qk_copy(g).wait()
            xn = xn_v[0]
            t0 = g * GT
            w = wqk_v[g]
            for i in range(GT):
                qk_v[t0 + i, HALO:HALO + TM, :] = jnp.dot(
                    xn, w[:, i * LANES:(i + 1) * LANES], preferred_element_type=_F32)
            return carry

        jax.lax.fori_loop(0, NG, group, 0)

    @pl.when(step == 0)
    def _():
        for n in range(NG, 16 // GT):
            qk_copy(n).wait()
        v_copy().wait()

    xn = xn_v[cur]
    for i in range(HT):
        qk_v[NT + HT + i, HALO:HALO + TM, :] = jnp.dot(xn, qk_tile(12 + i), preferred_element_type=_F32)
    _prep_cols(wv_v, wv_p, 0, D, "0" == "1")
    for i in range(NT):
        v_v[i, HALO:HALO + TM, :] = jnp.dot(xn, pltpu.bitcast(wv_p[i], _BF16), preferred_element_type=_F32)

    row = jax.lax.broadcasted_iota(jnp.int32, (RB, LANES), 0)
    scale = DH ** -0.5
    lane = jax.lax.broadcasted_iota(jnp.int32, (RB, LANES), 1)
    odd1 = (lane & 1) != 0
    odd2 = (lane & 2) != 0

    def attn_block(r0):
        grow = row + (step * TM + r0)
        qs = [qk_v[i, pl.ds(r0 + HALO, RB), :] for i in range(NT)]
        s = []
        for i in range(NT):
            kst = jnp.concatenate(
                [qk_v[NT + i, pl.ds(r0 + HALO - DIL * w, RB), :] for w in range(W)], axis=0)
            s.append(jnp.concatenate([qs[i]] * W, axis=0) * kst)
        lane_w = jax.lax.broadcasted_iota(jnp.int32, (W * RB, LANES), 1)
        for b in range(3):
            sh = 4 << b
            lo = (lane_w & sh) == 0
            if "r" in PERMS:
                s = [jnp.where(lo, s[2 * a], s[2 * a + 1])
                     + _xor_lanes(jnp.where(lo, s[2 * a + 1], s[2 * a]), sh)
                     for a in range(len(s) // 2)]
            else:
                s = [jnp.where(lo, s[2 * a] + pltpu.roll(s[2 * a], LANES - sh, 1),
                               s[2 * a + 1] + pltpu.roll(s[2 * a + 1], sh, 1))
                     for a in range(len(s) // 2)]
        acc = s[0]
        if "d" in PERMS:
            acc = acc + _xor_lanes(acc, 1)
            acc = acc + _xor_lanes(acc, 2)
        else:
            acc = acc + jnp.where((lane_w & 1) != 0, pltpu.roll(acc, 1, 1), pltpu.roll(acc, LANES - 1, 1))
            acc = acc + jnp.where((lane_w & 2) != 0, pltpu.roll(acc, 2, 1), pltpu.roll(acc, LANES - 2, 1))
        acc = acc * scale
        logits = []
        for w in range(W):
            l = acc[w * RB:(w + 1) * RB, :]
            if w > 0:
                l = jnp.where(grow >= DIL * w, l, -1e9)
            logits.append(l)
        mx = logits[0]
        for w in range(1, W):
            mx = jnp.maximum(mx, logits[w])
        es = [jnp.exp(l - mx) for l in logits]
        den = es[0]
        for w in range(1, W):
            den = den + es[w]
        inv = 1.0 / den
        ps = [e * inv for e in es]
        os_ = []
        for i in range(NT):
            acc = None
            for w in range(W):
                p = ps[w] * v_v[i, pl.ds(r0 + HALO - DIL * w, RB), :]
                acc = p if acc is None else acc + p
            os_.append(acc)
        os_ = _lane_butterfly(os_, "o" in PERMS)
        for i in range(NT):
            o_v[pl.ds(r0, RB), i * LANES:(i + 1) * LANES] = os_[i].astype(_BF16)

    def ffn_body(c, carry):
        @pl.when(step == 0)
        def _():
            for cp in f_copies(c):
                cp.wait()

        @pl.when(jnp.logical_and(c == 0, step < NSTEP - 1))
        def _():
            x_copy(step + 1).wait()

        base = pl.multiple_of(c * AR, AR)

        def part_f():
            xn = xn_v[cur]
            gate = jnp.dot(xn, w1_v[c], preferred_element_type=_F32)
            up = jnp.dot(xn, w3_v[c], preferred_element_type=_F32)
            h = (gate * jax.nn.sigmoid(gate) * up).astype(_BF16)
            d = jnp.dot(h, w2_v[c], preferred_element_type=_F32)
            acc_v[...] = jnp.where(c > 0, acc_v[...], 0.0) + d

        def part_a():
            for b in range(AR // RB):
                attn_block(base + b * RB)

        def part_l():
            nt = jnp.minimum(step + 1, NSTEP - 1)
            xn_v[nxt, pl.ds(base, AR), :] = _layernorm(x_v[nt, pl.ds(base, AR), :])

        for ch in "FAL":
            {"F": part_f, "A": part_a, "L": part_l}[ch]()
        return carry

    jax.lax.fori_loop(0, NC, ffn_body, 0)

    @pl.when(step == 0)
    def _():
        wo_copy().wait()

    OC = D // OCH

    def out_copy(t, ch):
        return pltpu.make_async_copy(
            out_v.at[ch], out_hbm.at[pl.ds(t * TM, TM), pl.ds(ch * OC, OC)],
            sems.at[_SEM_OUT + ch])

    @pl.when(step > 0)
    def _():
        for ch in range(OCH):
            out_copy(step - 1, ch).wait()

    def out_block():
        o = o_v[...]
        for ct in range(NT):
            cols = slice(ct * LANES, (ct + 1) * LANES)
            s = jnp.dot(o, wo_v[:, cols], preferred_element_type=_F32)
            ffn = acc_v[:, cols]
            g = ffn * jax.nn.sigmoid(ffn)
            per = NT // OCH
            ch, sub = ct // per, ct % per
            out_v[ch, :, sub * LANES:(sub + 1) * LANES] = (
                x_v[step, :, cols].astype(_F32) + s * g).astype(out_v.dtype)
            if sub == per - 1:
                out_copy(step, ch).start()

    @pl.when(step < NSTEP - 1)
    def _():
        out_block()
        halo(False)
        block12(nxt)

    @pl.when(step == NSTEP - 1)
    def _():
        out_block()

    @pl.when(step == NSTEP - 1)
    def _():
        for ch in range(OCH):
            out_copy(step, ch).wait()


@jax.jit
def pallas_recurrent_scan__sliding_local_dilated__glu_gated_swiglu__prompt_kernel(
    A_x: jax.Array,
    A_wqkv: jax.Array,
    A_wo: jax.Array,
    B_x: jax.Array,
    B_w1: jax.Array,
    B_w3: jax.Array,
    B_w2: jax.Array,
):
    x = A_x.reshape(S, D)
    any_spec = pl.BlockSpec(memory_space=pl.ANY)
    wp = pltpu.VMEM((NT, D // 2, LANES), _U32)
    out = pl.pallas_call(
        _kernel,
        grid=(NSTEP,),
        in_specs=[any_spec] * 6,
        out_specs=any_spec,
        out_shape=jax.ShapeDtypeStruct((S, D), A_x.dtype),
        scratch_shapes=[
            pltpu.VMEM((NSTEP, TM, D), _BF16),
            pltpu.VMEM((16 // GT, D, GT * LANES), _BF16),
            pltpu.VMEM((D, D), _BF16),
            pltpu.VMEM((D, D), _BF16),
            pltpu.VMEM((NC, D, FC), _BF16),
            pltpu.VMEM((NC, D, FC), _BF16),
            pltpu.VMEM((NC, FC, D), _BF16),
            wp,
            pltpu.VMEM((2, TM, D), _BF16),
            pltpu.VMEM((2 * NT, TM + HALO, LANES), _F32),
            pltpu.VMEM((NT, TM + HALO, LANES), _F32),
            pltpu.VMEM((TM, D), _BF16),
            pltpu.VMEM((TM, D), _F32),
            pltpu.VMEM((OCH, TM, D // OCH), _BF16),
            pltpu.SemaphoreType.DMA((_NSEM,)),
        ],
        compiler_params=pltpu.CompilerParams(
            dimension_semantics=("arbitrary",),
            vmem_limit_bytes=110 * 1024 * 1024,
        ),
        name="fused_block",
    )(x, A_wqkv, A_wo, B_w1, B_w3, B_w2)
    return out.reshape(A_x.shape)
```

```python
import jax
import jax.numpy as jnp
import jax.experimental.pallas as pl
import jax.experimental.pallas.tpu as pltpu

S = 2048
D = 1024
DH = 32
W = 8
DIL = 2
F = 3584
LANES = 128
NT = D // LANES
HALO = 16

TM = 512
NSTEP = S // TM
FC = 896
NC = F // FC
RB = 8
AR = TM // NC
XCH = 4
GT = 2
NQK = 2 * NT // GT
EARLY = 12
PR = 128

_F32 = jnp.float32
_BF16 = jnp.bfloat16
_U32 = jnp.uint32

_SEM_X = 0
_SEM_X0 = _SEM_X + NSTEP
_SEM_QK = _SEM_X0 + XCH
_SEM_V = _SEM_QK + NQK
_SEM_WO = _SEM_V + 1
_SEM_F = _SEM_WO + 1
_SEM_OUT = _SEM_F + 3 * NC
_NSEM = _SEM_OUT + NT


def _xor_lanes(x, k):
    lane = jax.lax.broadcasted_iota(jnp.int32, x.shape, 1)
    return jnp.take_along_axis(x, lane ^ k, axis=1)


def _lane_butterfly(tiles):
    s = list(tiles)
    lane = jax.lax.broadcasted_iota(jnp.int32, s[0].shape, 1)
    for bit in range(3):
        sh = 4 << bit
        lo = (lane & sh) == 0
        ns = list(s)
        for a in range(NT):
            if a & (1 << bit):
                continue
            c = a | (1 << bit)
            ns[a] = jnp.where(lo, s[a], pltpu.roll(s[c], sh, 1))
            ns[c] = jnp.where(lo, pltpu.roll(s[a], LANES - sh, 1), s[c])
        s = ns
    return s


def _layernorm(xb):
    x = xb.astype(_F32)
    mu = jnp.mean(x, axis=-1, keepdims=True)
    xc = x - mu
    var = jnp.mean(xc * xc, axis=-1, keepdims=True)
    return (xc * jax.lax.rsqrt(var + 1e-5)).astype(_BF16)


def _dot(a, b):
    return jnp.dot(a, b, preferred_element_type=_F32)


def _kernel(x_hbm, wqkv_hbm, wo_hbm, w1_hbm, w3_hbm, w2_hbm, out_hbm,
            x_v, wqk_v, wv_v, wo_v, w1_v, w3_v, w2_v, wv_p,
            xn_v, qk_v, v_v, o_v, acc_v, out_v, sems):
    step = pl.program_id(0)
    cur = step % 2
    nxt = 1 - cur
    rows = slice(HALO, HALO + TM)

    def x_copy(t):
        return pltpu.make_async_copy(
            x_hbm.at[pl.ds(t * TM, TM), :], x_v.at[t], sems.at[_SEM_X + t])

    def x0_copy(ch):
        n = TM // XCH
        return pltpu.make_async_copy(
            x_hbm.at[pl.ds(ch * n, n), :], x_v.at[0, pl.ds(ch * n, n), :],
            sems.at[_SEM_X0 + ch])

    def qk_copy(n):
        off = n * (GT * LANES)
        if not isinstance(n, int):
            off = pl.multiple_of(off, LANES)
        return pltpu.make_async_copy(
            wqkv_hbm.at[:, pl.ds(off, GT * LANES)], wqk_v.at[n], sems.at[_SEM_QK + n])

    def v_copy():
        return pltpu.make_async_copy(
            wqkv_hbm.at[:, pl.ds(2 * D, D)], wv_v, sems.at[_SEM_V])

    def wo_copy():
        return pltpu.make_async_copy(wo_hbm, wo_v, sems.at[_SEM_WO])

    def f_copies(c):
        off = c * FC
        if not isinstance(c, int):
            off = pl.multiple_of(off, LANES)
        sem = _SEM_F + 3 * c
        return [
            pltpu.make_async_copy(w1_hbm.at[:, pl.ds(off, FC)], w1_v.at[c], sems.at[sem]),
            pltpu.make_async_copy(w3_hbm.at[:, pl.ds(off, FC)], w3_v.at[c], sems.at[sem + 1]),
            pltpu.make_async_copy(w2_hbm.at[pl.ds(off, FC), :], w2_v.at[c], sems.at[sem + 2]),
        ]

    def out_copy(t, ct):
        return pltpu.make_async_copy(
            out_v.at[ct], out_hbm.at[pl.ds(t * TM, TM), pl.ds(ct * LANES, LANES)],
            sems.at[_SEM_OUT + ct])

    def qk_tile(t):
        return wqk_v[t // GT, :, (t % GT) * LANES:(t % GT + 1) * LANES]

    def set_halo(first):
        for buf, lo in ((qk_v, NT), (v_v, 0)):
            if first:
                buf[lo:lo + NT, 0:HALO, :] = jnp.zeros((NT, HALO, LANES), _F32)
            else:
                buf[lo:lo + NT, 0:HALO, :] = buf[lo:lo + NT, TM:TM + HALO, :]

    @pl.when(step == 0)
    def _():
        for ch in range(XCH):
            x0_copy(ch).start()
        for n in range(NQK):
            qk_copy(n).start()
        v_copy().start()
        for c in range(NC):
            for cp in f_copies(c):
                cp.start()
            if c == 0:
                x_copy(1).start()
            if c == 1:
                wo_copy().start()
                for t in range(2, NSTEP):
                    x_copy(t).start()
        n = TM // XCH
        for ch in range(XCH):
            x0_copy(ch).wait()
            xn_v[0, ch * n:(ch + 1) * n, :] = _layernorm(x_v[0, ch * n:(ch + 1) * n, :])

    @pl.when(step == 0)
    def _():
        set_halo(True)

        def group(g, carry):
            qk_copy(g).wait()
            xn = xn_v[0]
            w = wqk_v[g]
            for i in range(GT):
                qk_v[g * GT + i, rows, :] = _dot(xn, w[:, i * LANES:(i + 1) * LANES])
            return carry

        jax.lax.fori_loop(0, EARLY // GT, group, 0)

    @pl.when(step == 0)
    def _():
        for n in range(EARLY // GT, NQK):
            qk_copy(n).wait()
        v_copy().wait()

    xn = xn_v[cur]
    for t in range(EARLY, 2 * NT):
        qk_v[t, rows, :] = _dot(xn, qk_tile(t))
    for r in range(0, D, PR):
        outs = _lane_butterfly([
            pltpu.bitcast(wv_v[r:r + PR, j * LANES:(j + 1) * LANES], _U32) for j in range(NT)])
        for i in range(NT):
            wv_p[i, r // 2:(r + PR) // 2, :] = outs[i]
    for i in range(NT):
        v_v[i, rows, :] = _dot(xn, pltpu.bitcast(wv_p[i], _BF16))

    row = jax.lax.broadcasted_iota(jnp.int32, (RB, LANES), 0)
    lane_w = jax.lax.broadcasted_iota(jnp.int32, (W * RB, LANES), 1)
    scale = DH ** -0.5

    def attn_block(r0):
        grow = row + (step * TM + r0)
        s = []
        for i in range(NT):
            q = qk_v[i, pl.ds(r0 + HALO, RB), :]
            k = jnp.concatenate(
                [qk_v[NT + i, pl.ds(r0 + HALO - DIL * w, RB), :] for w in range(W)], axis=0)
            s.append(jnp.concatenate([q] * W, axis=0) * k)
        for bit in range(3):
            sh = 4 << bit
            lo = (lane_w & sh) == 0
            s = [jnp.where(lo, s[2 * a], s[2 * a + 1])
                 + _xor_lanes(jnp.where(lo, s[2 * a + 1], s[2 * a]), sh)
                 for a in range(len(s) // 2)]
        acc = s[0]
        acc = acc + _xor_lanes(acc, 1)
        acc = acc + _xor_lanes(acc, 2)
        acc = acc * scale
        logits = []
        for w in range(W):
            l = acc[w * RB:(w + 1) * RB, :]
            if w > 0:
                l = jnp.where(grow >= DIL * w, l, -1e9)
            logits.append(l)
        mx = logits[0]
        for w in range(1, W):
            mx = jnp.maximum(mx, logits[w])
        es = [jnp.exp(l - mx) for l in logits]
        den = es[0]
        for w in range(1, W):
            den = den + es[w]
        inv = 1.0 / den
        ps = [e * inv for e in es]
        os_ = []
        for i in range(NT):
            acc = None
            for w in range(W):
                p = ps[w] * v_v[i, pl.ds(r0 + HALO - DIL * w, RB), :]
                acc = p if acc is None else acc + p
            os_.append(acc)
        os_ = _lane_butterfly(os_)
        for i in range(NT):
            o_v[pl.ds(r0, RB), i * LANES:(i + 1) * LANES] = os_[i].astype(_BF16)

    def ffn_body(c, carry):
        @pl.when(step == 0)
        def _():
            for cp in f_copies(c):
                cp.wait()

        xn = xn_v[cur]
        gate = _dot(xn, w1_v[c])
        up = _dot(xn, w3_v[c])
        h = (gate * jax.nn.sigmoid(gate) * up).astype(_BF16)
        acc_v[...] = jnp.where(c > 0, acc_v[...], 0.0) + _dot(h, w2_v[c])

        base = pl.multiple_of(c * AR, AR)
        for b in range(AR // RB):
            attn_block(base + b * RB)

        nt = jnp.minimum(step + 1, NSTEP - 1)
        xn_v[nxt, pl.ds(base, AR), :] = _layernorm(x_v[nt, pl.ds(base, AR), :])
        return carry

    @pl.when(step < NSTEP - 1)
    def _():
        x_copy(step + 1).wait()

    jax.lax.fori_loop(0, NC, ffn_body, 0)

    @pl.when(step == 0)
    def _():
        wo_copy().wait()

    @pl.when(step > 0)
    def _():
        for ct in range(NT):
            out_copy(step - 1, ct).wait()

    def out_block():
        o = o_v[...]
        for ct in range(NT):
            cols = slice(ct * LANES, (ct + 1) * LANES)
            s = _dot(o, wo_v[:, cols])
            ffn = acc_v[:, cols]
            g = ffn * jax.nn.sigmoid(ffn)
            out_v[ct] = (x_v[step, :, cols].astype(_F32) + s * g).astype(out_v.dtype)
            out_copy(step, ct).start()

    @pl.when(step < NSTEP - 1)
    def _():
        out_block()
        set_halo(False)
        xn = xn_v[nxt]
        for t in range(EARLY):
            qk_v[t, rows, :] = _dot(xn, qk_tile(t))

    @pl.when(step == NSTEP - 1)
    def _():
        out_block()
        for ct in range(NT):
            out_copy(step, ct).wait()


@jax.jit
def pallas_recurrent_scan__sliding_local_dilated__glu_gated_swiglu__prompt_kernel(
    A_x: jax.Array,
    A_wqkv: jax.Array,
    A_wo: jax.Array,
    B_x: jax.Array,
    B_w1: jax.Array,
    B_w3: jax.Array,
    B_w2: jax.Array,
):
    x = A_x.reshape(S, D)
    any_spec = pl.BlockSpec(memory_space=pl.ANY)
    out = pl.pallas_call(
        _kernel,
        grid=(NSTEP,),
        in_specs=[any_spec] * 6,
        out_specs=any_spec,
        out_shape=jax.ShapeDtypeStruct((S, D), A_x.dtype),
        scratch_shapes=[
            pltpu.VMEM((NSTEP, TM, D), _BF16),
            pltpu.VMEM((NQK, D, GT * LANES), _BF16),
            pltpu.VMEM((D, D), _BF16),
            pltpu.VMEM((D, D), _BF16),
            pltpu.VMEM((NC, D, FC), _BF16),
            pltpu.VMEM((NC, D, FC), _BF16),
            pltpu.VMEM((NC, FC, D), _BF16),
            pltpu.VMEM((NT, D // 2, LANES), _U32),
            pltpu.VMEM((2, TM, D), _BF16),
            pltpu.VMEM((2 * NT, TM + HALO, LANES), _F32),
            pltpu.VMEM((NT, TM + HALO, LANES), _F32),
            pltpu.VMEM((TM, D), _BF16),
            pltpu.VMEM((TM, D), _F32),
            pltpu.VMEM((NT, TM, LANES), _BF16),
            pltpu.SemaphoreType.DMA((_NSEM,)),
        ],
        compiler_params=pltpu.CompilerParams(
            dimension_semantics=("arbitrary",),
            vmem_limit_bytes=110 * 1024 * 1024,
        ),
        name="fused_block",
    )(x, A_wqkv, A_wo, B_w1, B_w3, B_w2)
    return out.reshape(A_x.shape)
```

```python
import jax
import jax.numpy as jnp
import jax.experimental.pallas as pl
import jax.experimental.pallas.tpu as pltpu

S = 2048
D = 1024
DH = 32
W = 8
DIL = 2
F = 3584
LANES = 128
NT = D // LANES
HALO = 16

TM = 512
NSTEP = S // TM
FC = 896
NC = F // FC
RB = 8
AR = TM // NC
XCH = 4
GT = 2
NQK = 2 * NT // GT
EARLY = 12
PR = 128

_F32 = jnp.float32
_BF16 = jnp.bfloat16
_U32 = jnp.uint32

_SEM_X = 0
_SEM_X0 = _SEM_X + NSTEP
_SEM_QK = _SEM_X0 + XCH
_SEM_V = _SEM_QK + NQK
_SEM_WO = _SEM_V + 1
_SEM_F = _SEM_WO + 1
_SEM_OUT = _SEM_F + 3 * NC
_NSEM = _SEM_OUT + NT


def _xor_lanes(x, k):
    lane = jax.lax.broadcasted_iota(jnp.int32, x.shape, 1)
    return jnp.take_along_axis(x, lane ^ k, axis=1)


def _lane_butterfly(tiles):
    s = list(tiles)
    lane = jax.lax.broadcasted_iota(jnp.int32, s[0].shape, 1)
    for bit in range(3):
        sh = 4 << bit
        lo = (lane & sh) == 0
        ns = list(s)
        for a in range(NT):
            if a & (1 << bit):
                continue
            c = a | (1 << bit)
            ns[a] = jnp.where(lo, s[a], pltpu.roll(s[c], sh, 1))
            ns[c] = jnp.where(lo, pltpu.roll(s[a], LANES - sh, 1), s[c])
        s = ns
    return s


def _layernorm(xb):
    x = xb.astype(_F32)
    mu = jnp.mean(x, axis=-1, keepdims=True)
    xc = x - mu
    var = jnp.mean(xc * xc, axis=-1, keepdims=True)
    return (xc * jax.lax.rsqrt(var + 1e-5)).astype(_BF16)


def _silu(x):
    h = 0.5 * x
    return h + h * jnp.tanh(h)


def _dot(a, b):
    return jnp.dot(a, b, preferred_element_type=_F32)


def _kernel(x_hbm, wqkv_hbm, wo_hbm, w1_hbm, w3_hbm, w2_hbm, out_hbm,
            x_v, wqk_v, wv_v, wo_v, w1_v, w3_v, w2_v, wv_p,
            xn_v, qk_v, v_v, o_v, acc_v, out_v, sems):
    step = pl.program_id(0)
    cur = step % 2
    nxt = 1 - cur
    rows = slice(HALO, HALO + TM)

    def x_copy(t):
        return pltpu.make_async_copy(
            x_hbm.at[pl.ds(t * TM, TM), :], x_v.at[t], sems.at[_SEM_X + t])

    def x0_copy(ch):
        n = TM // XCH
        return pltpu.make_async_copy(
            x_hbm.at[pl.ds(ch * n, n), :], x_v.at[0, pl.ds(ch * n, n), :],
            sems.at[_SEM_X0 + ch])

    def qk_copy(n):
        off = n * (GT * LANES)
        if not isinstance(n, int):
            off = pl.multiple_of(off, LANES)
        return pltpu.make_async_copy(
            wqkv_hbm.at[:, pl.ds(off, GT * LANES)], wqk_v.at[n], sems.at[_SEM_QK + n])

    def v_copy():
        return pltpu.make_async_copy(
            wqkv_hbm.at[:, pl.ds(2 * D, D)], wv_v, sems.at[_SEM_V])

    def wo_copy():
        return pltpu.make_async_copy(wo_hbm, wo_v, sems.at[_SEM_WO])

    def f_copies(c):
        off = c * FC
        if not isinstance(c, int):
            off = pl.multiple_of(off, LANES)
        sem = _SEM_F + 3 * c
        return [
            pltpu.make_async_copy(w1_hbm.at[:, pl.ds(off, FC)], w1_v.at[c], sems.at[sem]),
            pltpu.make_async_copy(w3_hbm.at[:, pl.ds(off, FC)], w3_v.at[c], sems.at[sem + 1]),
            pltpu.make_async_copy(w2_hbm.at[pl.ds(off, FC), :], w2_v.at[c], sems.at[sem + 2]),
        ]

    def out_copy(t, ct):
        return pltpu.make_async_copy(
            out_v.at[ct], out_hbm.at[pl.ds(t * TM, TM), pl.ds(ct * LANES, LANES)],
            sems.at[_SEM_OUT + ct])

    def qk_tile(t):
        return wqk_v[t // GT, :, (t % GT) * LANES:(t % GT + 1) * LANES]

    def set_halo(first):
        for buf, lo in ((qk_v, NT), (v_v, 0)):
            if first:
                buf[lo:lo + NT, 0:HALO, :] = jnp.zeros((NT, HALO, LANES), _F32)
            else:
                buf[lo:lo + NT, 0:HALO, :] = buf[lo:lo + NT, TM:TM + HALO, :]

    @pl.when(step == 0)
    def _():
        for ch in range(XCH):
            x0_copy(ch).start()
        for n in range(NQK):
            qk_copy(n).start()
        v_copy().start()
        for c in range(NC):
            for cp in f_copies(c):
                cp.start()
            if c == 0:
                x_copy(1).start()
            if c == 1:
                wo_copy().start()
                for t in range(2, NSTEP):
                    x_copy(t).start()
        n = TM // XCH
        for ch in range(XCH):
            x0_copy(ch).wait()
            xn_v[0, ch * n:(ch + 1) * n, :] = _layernorm(x_v[0, ch * n:(ch + 1) * n, :])

    @pl.when(step == 0)
    def _():
        set_halo(True)

        def group(g, carry):
            qk_copy(g).wait()
            xn = xn_v[0]
            w = wqk_v[g]
            for i in range(GT):
                qk_v[g * GT + i, rows, :] = _dot(xn, w[:, i * LANES:(i + 1) * LANES])
            return carry

        jax.lax.fori_loop(0, EARLY // GT, group, 0)

    @pl.when(step == 0)
    def _():
        for n in range(EARLY // GT, NQK):
            qk_copy(n).wait()
        v_copy().wait()

    xn = xn_v[cur]
    for t in range(EARLY, 2 * NT):
        qk_v[t, rows, :] = _dot(xn, qk_tile(t))
    for r in range(0, D, PR):
        outs = _lane_butterfly([
            pltpu.bitcast(wv_v[r:r + PR, j * LANES:(j + 1) * LANES], _U32) for j in range(NT)])
        for i in range(NT):
            wv_p[i, r // 2:(r + PR) // 2, :] = outs[i]
    for i in range(NT):
        v_v[i, rows, :] = _dot(xn, pltpu.bitcast(wv_p[i], _BF16))

    row = jax.lax.broadcasted_iota(jnp.int32, (RB, LANES), 0)
    lane_w = jax.lax.broadcasted_iota(jnp.int32, (W * RB, LANES), 1)
    log2e = 1.4426950408889634
    scale = DH ** -0.5 * log2e
    masked = -1e9 * log2e

    def attn_block(r0):
        grow = row + (step * TM + r0)
        s = []
        for i in range(NT):
            q = qk_v[i, pl.ds(r0 + HALO, RB), :] * scale
            k = jnp.concatenate(
                [qk_v[NT + i, pl.ds(r0 + HALO - DIL * w, RB), :] for w in range(W)], axis=0)
            s.append(jnp.concatenate([q] * W, axis=0) * k)
        for bit in range(3):
            sh = 4 << bit
            lo = (lane_w & sh) == 0
            s = [jnp.where(lo, s[2 * a] + pltpu.roll(s[2 * a], LANES - sh, 1),
                           s[2 * a + 1] + pltpu.roll(s[2 * a + 1], sh, 1))
                 for a in range(len(s) // 2)]
        acc = s[0]
        acc = acc + _xor_lanes(acc, 1)
        acc = acc + _xor_lanes(acc, 2)
        logits = []
        for w in range(W):
            l = acc[w * RB:(w + 1) * RB, :]
            if w > 0:
                l = jnp.where(grow >= DIL * w, l, masked)
            logits.append(l)
        mx = logits[0]
        for w in range(1, W):
            mx = jnp.maximum(mx, logits[w])
        es = [jnp.exp2(l - mx) for l in logits]
        den = es[0]
        for w in range(1, W):
            den = den + es[w]
        inv = 1.0 / den
        os_ = []
        for i in range(NT):
            acc = None
            for w in range(W):
                p = es[w] * v_v[i, pl.ds(r0 + HALO - DIL * w, RB), :]
                acc = p if acc is None else acc + p
            os_.append(acc * inv)
        os_ = _lane_butterfly(os_)
        for i in range(NT):
            o_v[pl.ds(r0, RB), i * LANES:(i + 1) * LANES] = os_[i].astype(_BF16)

    def ffn_body(c, carry):
        @pl.when(step == 0)
        def _():
            for cp in f_copies(c):
                cp.wait()

        xn = xn_v[cur]
        gate = _dot(xn, w1_v[c])
        up = _dot(xn, w3_v[c])
        h = (_silu(gate) * up).astype(_BF16)
        acc_v[...] = jnp.where(c > 0, acc_v[...], 0.0) + _dot(h, w2_v[c])

        base = pl.multiple_of(c * AR, AR)
        for b in reversed(range(AR // RB)):
            attn_block(base + b * RB)

        nt = jnp.minimum(step + 1, NSTEP - 1)
        xn_v[nxt, pl.ds(base, AR), :] = _layernorm(x_v[nt, pl.ds(base, AR), :])
        return carry

    @pl.when(step < NSTEP - 1)
    def _():
        x_copy(step + 1).wait()

    jax.lax.fori_loop(0, NC, ffn_body, 0)

    @pl.when(step == 0)
    def _():
        wo_copy().wait()

    @pl.when(step > 0)
    def _():
        for ct in range(NT):
            out_copy(step - 1, ct).wait()

    def out_block():
        o = o_v[...]
        for ct in range(NT):
            cols = slice(ct * LANES, (ct + 1) * LANES)
            s = _dot(o, wo_v[:, cols])
            g = _silu(acc_v[:, cols])
            out_v[ct] = (x_v[step, :, cols].astype(_F32) + s * g).astype(out_v.dtype)
            out_copy(step, ct).start()

    @pl.when(step < NSTEP - 1)
    def _():
        set_halo(False)
        xn = xn_v[nxt]
        for t in range(EARLY):
            qk_v[t, rows, :] = _dot(xn, qk_tile(t))
        out_block()

    @pl.when(step == NSTEP - 1)
    def _():
        out_block()
        for ct in range(NT):
            out_copy(step, ct).wait()


@jax.jit
def pallas_recurrent_scan__sliding_local_dilated__glu_gated_swiglu__prompt_kernel(
    A_x: jax.Array,
    A_wqkv: jax.Array,
    A_wo: jax.Array,
    B_x: jax.Array,
    B_w1: jax.Array,
    B_w3: jax.Array,
    B_w2: jax.Array,
):
    x = A_x.reshape(S, D)
    any_spec = pl.BlockSpec(memory_space=pl.ANY)
    out = pl.pallas_call(
        _kernel,
        grid=(NSTEP,),
        in_specs=[any_spec] * 6,
        out_specs=any_spec,
        out_shape=jax.ShapeDtypeStruct((S, D), A_x.dtype),
        scratch_shapes=[
            pltpu.VMEM((NSTEP, TM, D), _BF16),
            pltpu.VMEM((NQK, D, GT * LANES), _BF16),
            pltpu.VMEM((D, D), _BF16),
            pltpu.VMEM((D, D), _BF16),
            pltpu.VMEM((NC, D, FC), _BF16),
            pltpu.VMEM((NC, D, FC), _BF16),
            pltpu.VMEM((NC, FC, D), _BF16),
            pltpu.VMEM((NT, D // 2, LANES), _U32),
            pltpu.VMEM((2, TM, D), _BF16),
            pltpu.VMEM((2 * NT, TM + HALO, LANES), _F32),
            pltpu.VMEM((NT, TM + HALO, LANES), _F32),
            pltpu.VMEM((TM, D), _BF16),
            pltpu.VMEM((TM, D), _F32),
            pltpu.VMEM((NT, TM, LANES), _BF16),
            pltpu.SemaphoreType.DMA((_NSEM,)),
        ],
        compiler_params=pltpu.CompilerParams(
            dimension_semantics=("arbitrary",),
            vmem_limit_bytes=110 * 1024 * 1024,
        ),
        name="fused_block",
    )(x, A_wqkv, A_wo, B_w1, B_w3, B_w2)
    return out.reshape(A_x.shape)
```

```python
import jax
import jax.numpy as jnp
import jax.experimental.pallas as pl
import jax.experimental.pallas.tpu as pltpu

S = 2048
D = 1024
DH = 32
W = 8
DIL = 2
F = 3584
LANES = 128
NT = D // LANES
HALO = 16

TM = 512
NSTEP = S // TM
FC = 896
NC = F // FC
RB = 8
AR = TM // NC
XCH = 4
GT = 2
NQK = 2 * NT // GT
EARLY = 12
PR = 128

_F32 = jnp.float32
_BF16 = jnp.bfloat16
_U32 = jnp.uint32

_SEM_X = 0
_SEM_X0 = _SEM_X + NSTEP
_SEM_QK = _SEM_X0 + XCH
_SEM_V = _SEM_QK + NQK
_SEM_WO = _SEM_V + 2
_SEM_F = _SEM_WO + 1
_SEM_OUT = _SEM_F + 3 * NC
_NSEM = _SEM_OUT + NT


def _xor_lanes(x, k):
    lane = jax.lax.broadcasted_iota(jnp.int32, x.shape, 1)
    return jnp.take_along_axis(x, lane ^ k, axis=1)


def _lane_butterfly(tiles):
    s = list(tiles)
    lane = jax.lax.broadcasted_iota(jnp.int32, s[0].shape, 1)
    for bit in range(3):
        sh = 4 << bit
        lo = (lane & sh) == 0
        ns = list(s)
        for a in range(NT):
            if a & (1 << bit):
                continue
            c = a | (1 << bit)
            ns[a] = jnp.where(lo, s[a], pltpu.roll(s[c], sh, 1))
            ns[c] = jnp.where(lo, pltpu.roll(s[a], LANES - sh, 1), s[c])
        s = ns
    return s


def _layernorm(xb):
    x = xb.astype(_F32)
    mu = jnp.mean(x, axis=-1, keepdims=True)
    xc = x - mu
    var = jnp.mean(xc * xc, axis=-1, keepdims=True)
    return (xc * jax.lax.rsqrt(var + 1e-5)).astype(_BF16)


def _silu(x):
    h = 0.5 * x
    return h + h * jnp.tanh(h)


def _dot(a, b):
    return jnp.dot(a, b, preferred_element_type=_F32)


def _kernel(x_hbm, wqkv_hbm, wo_hbm, w1_hbm, w3_hbm, w2_hbm, out_hbm,
            x_v, wqk_v, wv_v, wo_v, w1_v, w3_v, w2_v, wv_p,
            xn_v, qk_v, v_v, o_v, acc_v, out_v, sems):
    step = pl.program_id(0)
    cur = step % 2
    nxt = 1 - cur
    rows = slice(HALO, HALO + TM)

    def x_copy(t):
        return pltpu.make_async_copy(
            x_hbm.at[pl.ds(t * TM, TM), :], x_v.at[t], sems.at[_SEM_X + t])

    def x0_copy(ch):
        n = TM // XCH
        return pltpu.make_async_copy(
            x_hbm.at[pl.ds(ch * n, n), :], x_v.at[0, pl.ds(ch * n, n), :],
            sems.at[_SEM_X0 + ch])

    def qk_copy(n):
        off = n * (GT * LANES)
        if not isinstance(n, int):
            off = pl.multiple_of(off, LANES)
        return pltpu.make_async_copy(
            wqkv_hbm.at[:, pl.ds(off, GT * LANES)], wqk_v.at[n], sems.at[_SEM_QK + n])

    def v_copy(hf):
        n = D // 2
        return pltpu.make_async_copy(
            wqkv_hbm.at[pl.ds(hf * n, n), pl.ds(2 * D, D)], wv_v.at[pl.ds(hf * n, n), :],
            sems.at[_SEM_V + hf])

    def wo_copy():
        return pltpu.make_async_copy(wo_hbm, wo_v, sems.at[_SEM_WO])

    def f_copies(c):
        off = c * FC
        if not isinstance(c, int):
            off = pl.multiple_of(off, LANES)
        sem = _SEM_F + 3 * c
        return [
            pltpu.make_async_copy(w1_hbm.at[:, pl.ds(off, FC)], w1_v.at[c], sems.at[sem]),
            pltpu.make_async_copy(w3_hbm.at[:, pl.ds(off, FC)], w3_v.at[c], sems.at[sem + 1]),
            pltpu.make_async_copy(w2_hbm.at[pl.ds(off, FC), :], w2_v.at[c], sems.at[sem + 2]),
        ]

    def out_copy(t, ct):
        return pltpu.make_async_copy(
            out_v.at[ct], out_hbm.at[pl.ds(t * TM, TM), pl.ds(ct * LANES, LANES)],
            sems.at[_SEM_OUT + ct])

    def qk_tile(t):
        return wqk_v[t // GT, :, (t % GT) * LANES:(t % GT + 1) * LANES]

    def set_halo(first):
        for buf, lo in ((qk_v, NT), (v_v, 0)):
            if first:
                buf[lo:lo + NT, 0:HALO, :] = jnp.zeros((NT, HALO, LANES), _F32)
            else:
                buf[lo:lo + NT, 0:HALO, :] = buf[lo:lo + NT, TM:TM + HALO, :]

    @pl.when(step == 0)
    def _():
        for ch in range(XCH):
            x0_copy(ch).start()
        for n in range(NQK):
            qk_copy(n).start()
            if n == 1:
                v_copy(0).start()
            if n == 3:
                v_copy(1).start()
        for c in range(NC):
            for cp in f_copies(c):
                cp.start()
            if c == 0:
                x_copy(1).start()
            if c == 1:
                wo_copy().start()
                for t in range(2, NSTEP):
                    x_copy(t).start()
        n = TM // XCH
        for ch in range(XCH):
            x0_copy(ch).wait()
            xn_v[0, ch * n:(ch + 1) * n, :] = _layernorm(x_v[0, ch * n:(ch + 1) * n, :])

    @pl.when(step == 0)
    def _():
        set_halo(True)

        def qk_group(g):
            xn = xn_v[0]
            w = wqk_v[g]
            for i in range(GT):
                qk_v[g * GT + i, rows, :] = _dot(xn, w[:, i * LANES:(i + 1) * LANES])

        def group(g, carry):
            qk_copy(g).wait()
            qk_group(g)
            return carry

        def group_with_prep(g, carry):
            qk_copy(g).wait()

            @pl.when(g == 2)
            def _():
                v_copy(0).wait()

            @pl.when(g == 4)
            def _():
                v_copy(1).wait()

            qk_group(g)
            for sub in range(0, 256, PR):
                r = pl.multiple_of((g - 2) * 256 + sub, PR)
                outs = _lane_butterfly([
                    pltpu.bitcast(wv_v[pl.ds(r, PR), j * LANES:(j + 1) * LANES], _U32)
                    for j in range(NT)])
                r2 = pl.multiple_of((g - 2) * 128 + sub // 2, PR // 2)
                for i in range(NT):
                    wv_p[i, pl.ds(r2, PR // 2), :] = outs[i]
            return carry

        jax.lax.fori_loop(0, 2, group, 0)
        jax.lax.fori_loop(2, EARLY // GT, group_with_prep, 0)

    @pl.when(step == 0)
    def _():
        for n in range(EARLY // GT, NQK):
            qk_copy(n).wait()

    xn = xn_v[cur]
    for t in range(EARLY, 2 * NT):
        qk_v[t, rows, :] = _dot(xn, qk_tile(t))
    for i in range(NT):
        v_v[i, rows, :] = _dot(xn, pltpu.bitcast(wv_p[i], _BF16))

    row = jax.lax.broadcasted_iota(jnp.int32, (RB, LANES), 0)
    lane_w = jax.lax.broadcasted_iota(jnp.int32, (W * RB, LANES), 1)
    log2e = 1.4426950408889634
    scale = DH ** -0.5 * log2e
    masked = -1e9 * log2e

    def attn_block(r0):
        grow = row + (step * TM + r0)
        s = []
        for i in range(NT):
            q = qk_v[i, pl.ds(r0 + HALO, RB), :] * scale
            k = jnp.concatenate(
                [qk_v[NT + i, pl.ds(r0 + HALO - DIL * w, RB), :] for w in range(W)], axis=0)
            s.append(jnp.concatenate([q] * W, axis=0) * k)
        for bit in range(3):
            sh = 4 << bit
            lo = (lane_w & sh) == 0
            s = [jnp.where(lo, s[2 * a] + pltpu.roll(s[2 * a], LANES - sh, 1),
                           s[2 * a + 1] + pltpu.roll(s[2 * a + 1], sh, 1))
                 for a in range(len(s) // 2)]
        acc = s[0]
        acc = acc + _xor_lanes(acc, 1)
        acc = acc + _xor_lanes(acc, 2)
        logits = []
        for w in range(W):
            l = acc[w * RB:(w + 1) * RB, :]
            if w > 0:
                l = jnp.where(grow >= DIL * w, l, masked)
            logits.append(l)
        mx = logits[0]
        for w in range(1, W):
            mx = jnp.maximum(mx, logits[w])
        es = [jnp.exp2(l - mx) for l in logits]
        den = es[0]
        for w in range(1, W):
            den = den + es[w]
        inv = 1.0 / den
        os_ = []
        for i in range(NT):
            acc = None
            for w in range(W):
                p = es[w] * v_v[i, pl.ds(r0 + HALO - DIL * w, RB), :]
                acc = p if acc is None else acc + p
            os_.append(acc * inv)
        os_ = _lane_butterfly(os_)
        for i in range(NT):
            o_v[pl.ds(r0, RB), i * LANES:(i + 1) * LANES] = os_[i].astype(_BF16)

    def ffn_body(c, carry):
        @pl.when(step == 0)
        def _():
            for cp in f_copies(c):
                cp.wait()

        xn = xn_v[cur]
        gate = _dot(xn, w1_v[c])
        up = _dot(xn, w3_v[c])
        h = (_silu(gate) * up).astype(_BF16)
        acc_v[...] = jnp.where(c > 0, acc_v[...], 0.0) + _dot(h, w2_v[c])

        base = pl.multiple_of(c * AR, AR)
        for b in reversed(range(AR // RB)):
            attn_block(base + b * RB)

        nt = jnp.minimum(step + 1, NSTEP - 1)
        xn_v[nxt, pl.ds(base, AR), :] = _layernorm(x_v[nt, pl.ds(base, AR), :])
        return carry

    @pl.when(step < NSTEP - 1)
    def _():
        x_copy(step + 1).wait()

    jax.lax.fori_loop(0, NC, ffn_body, 0)

    @pl.when(step == 0)
    def _():
        wo_copy().wait()

    @pl.when(step > 0)
    def _():
        for ct in range(NT):
            out_copy(step - 1, ct).wait()

    def out_block():
        o = o_v[...]
        for ct in range(NT):
            cols = slice(ct * LANES, (ct + 1) * LANES)
            s = _dot(o, wo_v[:, cols])
            g = _silu(acc_v[:, cols])
            out_v[ct] = (x_v[step, :, cols].astype(_F32) + s * g).astype(out_v.dtype)
            out_copy(step, ct).start()

    @pl.when(step < NSTEP - 1)
    def _():
        set_halo(False)
        xn = xn_v[nxt]
        for t in range(EARLY):
            qk_v[t, rows, :] = _dot(xn, qk_tile(t))
        out_block()

    @pl.when(step == NSTEP - 1)
    def _():
        out_block()
        for ct in range(NT):
            out_copy(step, ct).wait()


@jax.jit
def pallas_recurrent_scan__sliding_local_dilated__glu_gated_swiglu__prompt_kernel(
    A_x: jax.Array,
    A_wqkv: jax.Array,
    A_wo: jax.Array,
    B_x: jax.Array,
    B_w1: jax.Array,
    B_w3: jax.Array,
    B_w2: jax.Array,
):
    x = A_x.reshape(S, D)
    any_spec = pl.BlockSpec(memory_space=pl.ANY)
    out = pl.pallas_call(
        _kernel,
        grid=(NSTEP,),
        in_specs=[any_spec] * 6,
        out_specs=any_spec,
        out_shape=jax.ShapeDtypeStruct((S, D), A_x.dtype),
        scratch_shapes=[
            pltpu.VMEM((NSTEP, TM, D), _BF16),
            pltpu.VMEM((NQK, D, GT * LANES), _BF16),
            pltpu.VMEM((D, D), _BF16),
            pltpu.VMEM((D, D), _BF16),
            pltpu.VMEM((NC, D, FC), _BF16),
            pltpu.VMEM((NC, D, FC), _BF16),
            pltpu.VMEM((NC, FC, D), _BF16),
            pltpu.VMEM((NT, D // 2, LANES), _U32),
            pltpu.VMEM((2, TM, D), _BF16),
            pltpu.VMEM((2 * NT, TM + HALO, LANES), _F32),
            pltpu.VMEM((NT, TM + HALO, LANES), _F32),
            pltpu.VMEM((TM, D), _BF16),
            pltpu.VMEM((TM, D), _F32),
            pltpu.VMEM((NT, TM, LANES), _BF16),
            pltpu.SemaphoreType.DMA((_NSEM,)),
        ],
        compiler_params=pltpu.CompilerParams(
            dimension_semantics=("arbitrary",),
            vmem_limit_bytes=110 * 1024 * 1024,
        ),
        name="fused_block",
    )(x, A_wqkv, A_wo, B_w1, B_w3, B_w2)
    return out.reshape(A_x.shape)
```
